```python
import jax
import jax.numpy as jnp

def _softmax(x, axis=-1):
    return jax.nn.softmax(x, axis=axis)

def _gelu(x):
    return jax.nn.gelu(x, approximate=True)

def _silu(x):
    return jax.nn.silu(x)

def _sigmoid(x):
    return jax.nn.sigmoid(x)

def _layernorm(x, axis=-1, eps=1e-05):
    m = jnp.mean(x, axis=axis, keepdims=True)
    v = jnp.var(x, axis=axis, keepdims=True)
    return (x - m) / jnp.sqrt(v + eps)

def _scatter_add(tgt, idx, src, axis=0):
    return tgt.at[idx].add(src)

def _segment_sum(src, seg, n):
    return jax.ops.segment_sum(src, seg, n)

class _Rng:

    def __init__(self, key):
        self._k = key

    def _next(self):
        self._k, sub = jax.random.split(self._k)
        return sub

    def normal(self, shape):
        return jax.random.normal(self._next(), shape, dtype=jnp.bfloat16)

    def randint(self, lo, hi, shape):
        return jax.random.randint(self._next(), shape, lo, hi, dtype=jnp.int32)

    def uniform(self, shape, lo=0.0, hi=1.0):
        return jax.random.uniform(self._next(), shape, jnp.bfloat16, lo, hi)

    def permutation(self, n):
        return jax.random.permutation(self._next(), n)
kernel_name = 'interleave_layers__memory_aug_recurrent_mem_tr__glu_gated_glu__prompt'

def setup_inputs():
    _rng = _Rng(jax.random.key(int.from_bytes(__import__("os").urandom(4), "little")))
    _w = lambda a: (lambda t: t.astype(jnp.bfloat16) if jnp.issubdtype(t.dtype, jnp.floating) else t)(jnp.asarray(a))

    def _A_setup():
        B, S, Dm = (1, 2048, 1024)
        H, Dh = (32, 128)
        M, seg = (8, 32)
        seg = min(seg, S)
        S = S // seg * seg
        return {'x': _w((lambda *s: _rng.normal(s) * 0.05)(B, S, Dm)), 'mem0': _w((lambda *s: _rng.normal(s) * 0.05)(B, M, Dm)), 'Wq': _w((lambda *s: _rng.normal(s) * 0.05)(Dm, H, Dh) * Dm ** (-0.5)), 'Wk': _w((lambda *s: _rng.normal(s) * 0.05)(Dm, H, Dh) * Dm ** (-0.5)), 'Wv': _w((lambda *s: _rng.normal(s) * 0.05)(Dm, H, Dh) * Dm ** (-0.5)), 'Wo': _w((lambda *s: _rng.normal(s) * 0.05)(H, Dh, Dm) * (H * Dh) ** (-0.5)), 'seg_len': seg}
    _A_in = _A_setup()

    def _B_setup():
        B, S, D, F = (1, 2048, 1024, 3584)
        return {'x': _w((lambda *s: _rng.normal(s) * 0.05)(B, S, D)), 'w_gate': _w((lambda *s: _rng.normal(s) * 0.05)(D, F)), 'w_up': _w((lambda *s: _rng.normal(s) * 0.05)(D, F)), 'w_down': _w((lambda *s: _rng.normal(s) * 0.05)(F, D))}
    _B_in = _B_setup()
    return {'A_x': _A_in['x'], 'A_mem0': _A_in['mem0'], 'A_Wq': _A_in['Wq'], 'A_Wk': _A_in['Wk'], 'A_Wv': _A_in['Wv'], 'A_Wo': _A_in['Wo'], 'A_seg_len': _A_in['seg_len'], 'B_x': _B_in['x'], 'B_w_gate': _B_in['w_gate'], 'B_w_up': _B_in['w_up'], 'B_w_down': _B_in['w_down']}

def reference(A_x, A_mem0, A_Wq, A_Wk, A_Wv, A_Wo, A_seg_len, B_x, B_w_gate, B_w_up, B_w_down):

    def _A_ref(x, mem0, Wq, Wk, Wv, Wo, seg_len):
        B, S, Dm = x.shape
        H, Dh = (Wq.shape[1], Wq.shape[2])
        M = mem0.shape[1]
        scale = Dh ** (-0.5)
        n_seg = S // seg_len
        L = M + seg_len
        idx = jnp.arange(L)
        mask = (idx[:, None] < M) | (idx[:, None] >= idx[None, :])
        mem = mem0
        outs = []
        for s in range(n_seg):
            xs = x[:, s * seg_len:(s + 1) * seg_len, :].copy()
            h = jnp.concatenate([mem, xs], axis=1)
            q = jnp.einsum('btd,dhe->bhte', h, Wq)
            k = jnp.einsum('btd,dhe->bhte', h, Wk)
            v = jnp.einsum('btd,dhe->bhte', h, Wv)
            scores = jnp.einsum('bhqe,bhke->bhqk', q, k) * scale
            scores = jnp.where(mask[None, None], scores, -1000000000.0)
            p = _softmax(scores, axis=-1)
            o = jnp.einsum('bhqk,bhke->bhqe', p, v)
            o = jnp.einsum('bhte,hed->btd', o, Wo)
            mem = o[:, :M, :].copy()
            outs.append(o[:, M:, :])
        return jnp.concatenate(outs, axis=1)

    def _B_ref(x, w_gate, w_up, w_down):
        g = jnp.einsum('bsd,df->bsf', x, w_gate)
        u = jnp.einsum('bsd,df->bsf', x, w_up)
        h = _sigmoid(g) * u
        return jnp.einsum('bsf,fd->bsd', h, w_down)
    x = A_x
    x = x + _A_ref(_layernorm(x, axis=-1), A_mem0, A_Wq, A_Wk, A_Wv, A_Wo, A_seg_len)
    x = x + _B_ref(_layernorm(x, axis=-1), B_w_gate, B_w_up, B_w_down)
    x = x + _A_ref(_layernorm(x, axis=-1), A_mem0, A_Wq, A_Wk, A_Wv, A_Wo, A_seg_len)
    x = x + _B_ref(_layernorm(x, axis=-1), B_w_gate, B_w_up, B_w_down)
    return x
```

```python
import functools
import jax
import jax.numpy as jnp
import jax.experimental.pallas as pl
import jax.experimental.pallas.tpu as pltpu

F32 = jnp.float32
BF16 = jnp.bfloat16
U32 = jnp.uint32

S, D, H, DH, M, SEG, FF = 2048, 1024, 32, 128, 8, 32, 3584
NSEG = S // SEG
KT = D // 128
FT = FF // 128
RA = 2 * M + 2 * SEG
RB = 2 * SEG
NSTEP = NSEG + 3
DCH = 128
NRING = 4
XR = 4
EPS = 1e-5
NEG_REF = -1e9


def _ln(x):
    m = jnp.mean(x, axis=-1, keepdims=True)
    xc = x - m
    v = jnp.mean(xc * xc, axis=-1, keepdims=True)
    return xc * jax.lax.rsqrt(v + EPS)


def _pack(x):
    return pltpu.bitcast(x, U32)


def _unpack(x):
    return pltpu.bitcast(x, BF16)


def _cat(ref, n):
    return jnp.concatenate([_unpack(ref[k]) for k in range(n)], axis=1)


def _store_tiles(ref, r0, x):
    rows = x.shape[0]
    for k in range(KT):
        ref[k, r0 // 2:(r0 + rows) // 2, :] = _pack(x[:, k * 128:(k + 1) * 128])


def _recip(x):
    r = pl.reciprocal(x, approx=True)
    return r * (2.0 - x * r)


def _dot(a, b):
    return jnp.dot(a, b, preferred_element_type=F32)


def _fill(rows_layer, rows_pos, n):
    r = jax.lax.broadcasted_iota(jnp.int32, (n, n), 0)
    c = jax.lax.broadcasted_iota(jnp.int32, (n, n), 1)
    same = rows_layer(r) == rows_layer(c)
    ok = (rows_pos(r) < M) | (rows_pos(r) >= rows_pos(c))
    return jnp.where(same, jnp.where(ok, 0.0, NEG_REF), -jnp.inf).astype(F32)


def _kernel(x_hbm, mem0_hbm, wq_hbm, wk_hbm, wv_hbm, wo_hbm, wg_hbm, wu_hbm, wd_hbm,
            out_hbm,
            xr_s, mem0_s, wq_s, wk_s, wv_s, wo_s, wg_s, wu_s, wd_s,
            st3, sto, stg, stu, std,
            ha_s, hb_s, o_s, act_s, x1a_s, x2_s, x2a_s, xb_s, ost_s, mfill_s,
            sem_x, sem_m, sem_st, sem_w, sem_o):
    scale = DH ** -0.5

    def x_copy(seg):
        return pltpu.make_async_copy(x_hbm.at[pl.ds(pl.multiple_of(seg * SEG, SEG), SEG)],
                                     xr_s.at[seg % XR], sem_x.at[seg % XR])

    def out_copy(t):
        seg = t - 3
        return pltpu.make_async_copy(ost_s.at[t % 2],
                                     out_hbm.at[pl.ds(pl.multiple_of(seg * SEG, SEG), SEG)], sem_o.at[t % 2])

    def whole(src, dst, i):
        return pltpu.make_async_copy(src, dst, sem_w.at[i])
    c_wo, c_wg, c_wu, c_wd = whole(wo_hbm, sto, 0), whole(wg_hbm, stg, 1), whole(wu_hbm, stu, 2), whole(wd_hbm, std, 3)

    def conv_cols(src, dst, nrows, ntile):
        def body(c, carry):
            blk = src[pl.ds(pl.multiple_of(c * DCH, DCH), DCH), :]
            rows = pl.ds(pl.multiple_of(c * (DCH // 2), DCH // 2), DCH // 2)
            for j in range(ntile):
                dst[j, rows, :] = _pack(blk[:, j * 128:(j + 1) * 128])
            return carry
        jax.lax.fori_loop(0, nrows // DCH, body, 0)

    cm = pltpu.make_async_copy(mem0_hbm, mem0_s, sem_m)
    cm.start()
    for s in range(3):
        x_copy(s).start()

    nch = D // DCH
    qkv_src = [wq_hbm, wk_hbm, wv_hbm]
    qkv_dst = [wq_s, wk_s, wv_s]

    def st_copy(w, c, slot):
        return pltpu.make_async_copy(qkv_src[w].at[pl.ds(pl.multiple_of(c * DCH, DCH), DCH)], st3.at[slot], sem_st.at[slot])

    for i in range(NRING - 1):
        st_copy(0, i, i).start()
    for w in range(3):
        def body(c, carry, w=w):
            g = w * nch + c
            nxt = c + NRING - 1
            slot_n = (g + NRING - 1) % NRING

            @pl.when(nxt < nch)
            def _():
                st_copy(w, nxt, slot_n).start()
            if w < 2:
                @pl.when(nxt >= nch)
                def _():
                    st_copy(w + 1, nxt - nch, slot_n).start()
            else:
                @pl.when(nxt == nch)
                def _():
                    c_wo.start()
            st_copy(w, c, g % NRING).wait()
            t = jnp.swapaxes(st3[g % NRING], 0, 1)
            rows = pl.ds(pl.multiple_of(c * (DCH // 2), DCH // 2), DCH // 2)
            for h in range(H):
                qkv_dst[w][h, rows, :] = _pack(t[h])
            return carry
        jax.lax.fori_loop(0, nch, body, 0)

    mfill_s[...] = _fill(lambda i: jnp.where(i < 2 * M, i // M, (i - 2 * M) // SEG),
                         lambda i: jnp.where(i < 2 * M, i % M, M + (i - 2 * M) % SEG), RA)
    cm.wait()
    x_copy(0).wait()
    x_copy(1).wait()
    x2a_s[...] = jnp.zeros_like(x2a_s)
    x2_s[...] = jnp.zeros_like(x2_s)
    x1a_s[...] = jnp.zeros_like(x1a_s)
    m0 = mem0_s[...]
    _store_tiles(ha_s, 0, jnp.concatenate([m0, m0], axis=0))
    _store_tiles(ha_s, 2 * M, _ln(xr_s[0].astype(F32)).astype(BF16))
    _store_tiles(ha_s, 2 * M + SEG, jnp.zeros((SEG, D), BF16))

    def attention_phase(ha, fill, filler, mid=None):
        allowed = fill == 0.0
        rows = ha.shape[0]

        def qkv(h):
            q = _dot(ha, _unpack(wq_s[h]))
            kk = _dot(ha, _unpack(wk_s[h]))
            v = _dot(ha, _unpack(wv_s[h]))
            return (q * scale).astype(BF16), kk.astype(BF16), v.astype(BF16)

        def probs(q, kk):
            s = jax.lax.dot_general(q, kk, (((1,), (1,)), ((), ())), preferred_element_type=F32)
            s = jnp.where(allowed, s, fill)
            p = jnp.exp(s - jnp.max(s, axis=-1, keepdims=True))
            return (p * _recip(jnp.sum(p, axis=-1, keepdims=True))).astype(BF16)

        qs, ps = {}, {}
        for i in range(H + 2):
            if i < H:
                qs[i] = qkv(i)
            else:
                filler(i - H)
            if 0 <= i - 1 < H:
                ps[i - 1] = probs(qs[i - 1][0], qs[i - 1][1])
            if 0 <= i - 2 < H:
                o = _dot(ps.pop(i - 2), qs.pop(i - 2)[2])
                o_s[i - 2, 0:rows // 2, :] = _pack(o.astype(BF16))
            if mid is not None and i == H // 2:
                mid()

    def out_proj(rows):
        o = jnp.concatenate([_unpack(o_s[h, 0:rows // 2, :]) for h in range(H)], axis=1)
        return jnp.concatenate([_dot(o, _unpack(wo_s[n])) for n in range(KT)], axis=1)

    def glu_chunk(hb, j):
        rows = hb.shape[0]
        g = _dot(hb, _unpack(wg_s[j]))
        u = _dot(hb, _unpack(wu_s[j]))
        act_s[j, 0:rows // 2, :] = _pack((jax.nn.sigmoid(g) * u).astype(BF16))

    def glu_down(rows):
        act = jnp.concatenate([_unpack(act_s[j, 0:rows // 2, :]) for j in range(FT)], axis=1)
        return jnp.concatenate([_dot(act, _unpack(wd_s[n])) for n in range(KT)], axis=1)

    def xseg(seg):
        return xr_s[seg % XR].astype(F32)

    def full_step(t):
        x1a = x1a_s[...]
        x2a = x2a_s[...]
        _store_tiles(hb_s, 0, _ln(x1a).astype(BF16))
        _store_tiles(hb_s, SEG, _ln(x2a).astype(BF16))
        ha = _cat(ha_s, KT)
        hb = _cat(hb_s, KT)

        def filler(i):
            glu_chunk(hb, 2 * i)
            glu_chunk(hb, 2 * i + 1)
        attention_phase(ha, mfill_s[...], filler)
        for j in range(4, FT):
            glu_chunk(hb, j)
        z = glu_down(RB)

        xin = xseg(jnp.minimum(t, NSEG - 1))
        x2_old = x2_s[...]
        x2_new = x1a + z[0:SEG]
        x2_s[...] = x2_new
        ost_s[t % 2] = (x2a + z[SEG:RB]).astype(BF16)
        n1 = _ln(xseg(jnp.minimum(t + 1, NSEG - 1))).astype(BF16)
        n2 = _ln(x2_new).astype(BF16)

        y = out_proj(RA)
        _store_tiles(ha_s, 0, y[0:2 * M].astype(BF16))
        _store_tiles(ha_s, 2 * M, n1)
        _store_tiles(ha_s, 2 * M + SEG, n2)
        x1a_s[...] = xin + y[2 * M:2 * M + SEG]
        x2a_s[...] = x2_old + y[2 * M + SEG:RA]

    def half_step(t):
        late = t > 2
        li = late.astype(jnp.int32)
        xb_s[...] = jnp.where(late, x2a_s[...], x1a_s[...])

        @pl.when(t < NSTEP - 1)
        def _():
            RH = 2 * M + SEG
            tok0 = pl.multiple_of(M + (SEG // 2) * li, M)
            ha = jnp.concatenate(
                [jnp.concatenate([_unpack(ha_s[k, 0:M, :]), _unpack(ha_s[k, pl.ds(tok0, SEG // 2), :])], axis=0)
                 for k in range(KT)], axis=1)
            fill = _fill(lambda i: jnp.where(i < 2 * M, i // M, li),
                         lambda i: jnp.where(i < 2 * M, i % M, M + i - 2 * M), RH)

            def mid():
                @pl.when(t == 0)
                def _():
                    c_wg.start()
            attention_phase(ha, fill, lambda i: None, mid)

            @pl.when(t == 0)
            def _():
                c_wo.wait()
                c_wu.start()
                c_wd.start()
                conv_cols(sto, wo_s, H * DH, KT)
            y = out_proj(RH)
            res = jnp.where(late, x2_s[...], xseg(jnp.minimum(t, 1))) + y[2 * M:RH]

            @pl.when(jnp.logical_not(late))
            def _():
                m0f = mem0_s[...].astype(F32)
                _store_tiles(ha_s, 0, jnp.concatenate([y[0:M], m0f], axis=0).astype(BF16))
                _store_tiles(ha_s, 2 * M, _ln(xseg(t + 1)).astype(BF16))
                x1a_s[...] = res

            @pl.when(late)
            def _():
                x2a_s[...] = res

        @pl.when(t == 1)
        def _():
            c_wg.wait()
            conv_cols(stg, wg_s, D, FT)
            c_wu.wait()
            conv_cols(stu, wu_s, D, FT)
            c_wd.wait()
            conv_cols(std, wd_s, FF, KT)

        @pl.when(t >= 1)
        def _():
            xb = xb_s[...]
            hb = _ln(xb).astype(BF16)
            for j in range(FT):
                glu_chunk(hb, j)
            res = xb + glu_down(SEG)

            @pl.when(jnp.logical_not(late))
            def _():
                x2_s[...] = res
                _store_tiles(ha_s, 2 * M + SEG, _ln(res).astype(BF16))

            @pl.when(late)
            def _():
                ost_s[t % 2] = res.astype(BF16)

    def step(t, carry):
        @pl.when(t >= 5)
        def _():
            out_copy(t - 2).wait()

        @pl.when(jnp.logical_and(t >= 1, t + 1 < NSEG))
        def _():
            x_copy(t + 1).wait()

        @pl.when(t + 3 < NSEG)
        def _():
            x_copy(t + 3).start()

        is_half = jnp.logical_or(t < 2, t > NSEG)

        @pl.when(is_half)
        def _():
            half_step(t)

        @pl.when(jnp.logical_not(is_half))
        def _():
            full_step(t)

        @pl.when(t >= 3)
        def _():
            out_copy(t).start()
        return carry

    jax.lax.fori_loop(0, NSTEP, step, 0)
    out_copy(NSTEP - 2).wait()
    out_copy(NSTEP - 1).wait()


@jax.jit
def pallas_interleave_layers__memory_aug_recurrent_mem_tr__glu_gated_glu__prompt_kernel(A_x, A_mem0, A_Wq, A_Wk, A_Wv, A_Wo, A_seg_len, B_x, B_w_gate, B_w_up, B_w_down):
    x = A_x.reshape(S, D)
    mem0 = A_mem0.reshape(M, D)
    wo = A_Wo.reshape(H * DH, D)
    any_spec = pl.BlockSpec(memory_space=pl.ANY)
    out = pl.pallas_call(
        _kernel,
        out_shape=jax.ShapeDtypeStruct((S, D), BF16),
        in_specs=[any_spec] * 9,
        out_specs=any_spec,
        scratch_shapes=[
            pltpu.VMEM((XR, SEG, D), BF16),
            pltpu.VMEM((M, D), BF16),
            pltpu.VMEM((H, D // 2, DH), U32),
            pltpu.VMEM((H, D // 2, DH), U32),
            pltpu.VMEM((H, D // 2, DH), U32),
            pltpu.VMEM((KT, H * DH // 2, 128), U32),
            pltpu.VMEM((FT, D // 2, 128), U32),
            pltpu.VMEM((FT, D // 2, 128), U32),
            pltpu.VMEM((KT, FF // 2, 128), U32),
            pltpu.VMEM((NRING, DCH, H, DH), BF16),
            pltpu.VMEM((H * DH, D), BF16),
            pltpu.VMEM((D, FF), BF16),
            pltpu.VMEM((D, FF), BF16),
            pltpu.VMEM((FF, D), BF16),
            pltpu.VMEM((KT, RA // 2, 128), U32),
            pltpu.VMEM((KT, RB // 2, 128), U32),
            pltpu.VMEM((H, RA // 2, 128), U32),
            pltpu.VMEM((FT, RB // 2, 128), U32),
            pltpu.VMEM((SEG, D), F32),
            pltpu.VMEM((SEG, D), F32),
            pltpu.VMEM((SEG, D), F32),
            pltpu.VMEM((SEG, D), F32),
            pltpu.VMEM((2, SEG, D), BF16),
            pltpu.VMEM((RA, RA), F32),
            pltpu.SemaphoreType.DMA((XR,)),
            pltpu.SemaphoreType.DMA,
            pltpu.SemaphoreType.DMA((NRING,)),
            pltpu.SemaphoreType.DMA((4,)),
            pltpu.SemaphoreType.DMA((2,)),
        ],
        compiler_params=pltpu.CompilerParams(vmem_limit_bytes=120 * 1024 * 1024),
    )(x, mem0, A_Wq, A_Wk, A_Wv, wo, B_w_gate, B_w_up, B_w_down)
    return out.reshape(1, S, D)
```

```python
import functools
import jax
import jax.numpy as jnp
import jax.experimental.pallas as pl
import jax.experimental.pallas.tpu as pltpu

F32 = jnp.float32
BF16 = jnp.bfloat16
U32 = jnp.uint32

S, D, H, DH, M, SEG, FF = 2048, 1024, 32, 128, 8, 32, 3584
NSEG = S // SEG
KT = D // 128
FT = FF // 128
RA = 2 * M + 2 * SEG
RB = 2 * SEG
NSTEP = NSEG + 3
DCH = 128
NCH = D // DCH
NPRE = 9
PRE0 = 2
XR = 16
XPF = 12
HG = 8
EPS = 1e-5
NEG_REF = -1e9


def _ln(x):
    m = jnp.mean(x, axis=-1, keepdims=True)
    xc = x - m
    v = jnp.mean(xc * xc, axis=-1, keepdims=True)
    return xc * jax.lax.rsqrt(v + EPS)


def _pack(x):
    return pltpu.bitcast(x, U32)


def _unpack(x):
    return pltpu.bitcast(x, BF16)


def _cat(ref, n):
    return jnp.concatenate([_unpack(ref[k]) for k in range(n)], axis=1)


def _store_tiles(ref, r0, x):
    rows = x.shape[0]
    for k in range(KT):
        ref[k, r0 // 2:(r0 + rows) // 2, :] = _pack(x[:, k * 128:(k + 1) * 128])


def _recip(x):
    r = pl.reciprocal(x, approx=True)
    return r * (2.0 - x * r)


def _dot(a, b):
    return jnp.dot(a, b, preferred_element_type=F32)


def _fill(rows_layer, rows_pos, n):
    r = jax.lax.broadcasted_iota(jnp.int32, (n, n), 0)
    c = jax.lax.broadcasted_iota(jnp.int32, (n, n), 1)
    same = rows_layer(r) == rows_layer(c)
    ok = (rows_pos(r) < M) | (rows_pos(r) >= rows_pos(c))
    return jnp.where(same, jnp.where(ok, 0.0, NEG_REF), -jnp.inf).astype(F32)


def _kernel(x_hbm, mem0_hbm, wq_hbm, wk_hbm, wv_hbm, wo_hbm, wg_hbm, wu_hbm, wd_hbm,
            out_hbm,
            xr_s, mem0_s, wq_s, wk_s, wv_s, wo_s, wg_s, wu_s, wd_s,
            st3, sto, stg, stu, std,
            ha_s, hb_s, hp_s, pre_s, o_s, act_s, x1a_s, x2_s, x2a_s, xb_s, ost_s, mfill_s,
            sem_x, sem_m, sem_st, sem_w, sem_o):
    scale = DH ** -0.5

    def x_copy(seg):
        return pltpu.make_async_copy(x_hbm.at[pl.ds(pl.multiple_of(seg * SEG, SEG), SEG)],
                                     xr_s.at[seg % XR], sem_x.at[seg % XR])

    def out_copy(t):
        seg = t - 3
        return pltpu.make_async_copy(ost_s.at[t % 2],
                                     out_hbm.at[pl.ds(pl.multiple_of(seg * SEG, SEG), SEG)], sem_o.at[t % 2])

    def whole(src, dst, i):
        return pltpu.make_async_copy(src, dst, sem_w.at[i])
    c_wo, c_wg, c_wu, c_wd = whole(wo_hbm, sto, 0), whole(wg_hbm, stg, 1), whole(wu_hbm, stu, 2), whole(wd_hbm, std, 3)

    def conv_cols(src, dst, nrows, ntile):
        def body(c, carry):
            blk = src[pl.ds(pl.multiple_of(c * DCH, DCH), DCH), :]
            rows = pl.ds(pl.multiple_of(c * (DCH // 2), DCH // 2), DCH // 2)
            for j in range(ntile):
                dst[j, rows, :] = _pack(blk[:, j * 128:(j + 1) * 128])
            return carry
        jax.lax.fori_loop(0, nrows // DCH, body, 0)

    cm = pltpu.make_async_copy(mem0_hbm, mem0_s, sem_m)
    cm.start()
    for s in range(XPF):
        x_copy(s).start()

    qkv_src = [wq_hbm, wk_hbm, wv_hbm]
    qkv_dst = [wq_s, wk_s, wv_s]

    def st_copy(w, c):
        slot = (w % 2) * NCH + c
        return pltpu.make_async_copy(qkv_src[w].at[pl.ds(pl.multiple_of(c * DCH, DCH), DCH)], st3.at[slot], sem_st.at[slot])

    SUB = 16
    NSUB = DCH // SUB

    def convert_sub(w, c, s):
        x = pltpu.bitcast(st3[(w % 2) * NCH + c, s * SUB:(s + 1) * SUB], U32)
        x = x.reshape(SUB // 2, 2, H // 2, DH)
        a, b = x[:, 0], x[:, 1]
        lo = jnp.swapaxes((a & jnp.uint32(0xFFFF)) | (b << 16), 0, 1)
        hi = jnp.swapaxes((a >> 16) | (b & jnp.uint32(0xFFFF0000)), 0, 1)
        rows = pl.ds(pl.multiple_of(c * (DCH // 2) + s * (SUB // 2), SUB // 2), SUB // 2)
        for i in range(H // 2):
            qkv_dst[w][2 * i, rows, :] = lo[i]
            qkv_dst[w][2 * i + 1, rows, :] = hi[i]

    def convert(w, c):
        for s in range(NSUB):
            convert_sub(w, c, s)

    LOOK = NCH // 2
    for c in range(LOOK):
        st_copy(0, c).start()
    for s in range(PRE0 + NPRE):
        x_copy(s).wait()
    for s in range(NPRE):
        _store_tiles(hp_s, s * SEG, _ln(xr_s[PRE0 + s].astype(F32)).astype(BF16))

    def conv_body(c, carry):
        @pl.when(c < LOOK)
        def _():
            st_copy(0, c + LOOK).start()

        @pl.when(c >= LOOK)
        def _():
            st_copy(1, c - LOOK).start()
        st_copy(0, c).wait()
        convert(0, c)
        return carry
    jax.lax.fori_loop(0, NCH, conv_body, 0)
    for c in range(LOOK, NCH):
        st_copy(1, c).start()
    for c in range(NCH):
        st_copy(2, c).start()

    hooks = {(1, 2): c_wo, (2, 0): c_wg, (2, 1): c_wu, (2, 3): c_wd}
    NG = H // HG
    CPG = NCH // NG
    for w in range(3):
        def pre_body(g, carry, w=w):
            for (hw, hg), cp in hooks.items():
                if hw == w:
                    @pl.when(g == hg)
                    def _(cp=cp):
                        cp.start()
            if w < 2:
                for i in range(CPG):
                    st_copy(w + 1, g * CPG + i).wait()
            hp = _cat(hp_s, KT)
            for j in range(HG):
                h = g * HG + j
                r = _dot(hp, _unpack(qkv_dst[w][h]))
                if w == 0:
                    r = r * scale
                r = _pack(r.astype(BF16))
                for s in range(NPRE):
                    pre_s[s, w, h] = r[s * (SEG // 2):(s + 1) * (SEG // 2)]
                if w < 2:
                    per = CPG * NSUB // HG
                    for k in range(j * per, (j + 1) * per):
                        convert_sub(w + 1, g * CPG + k // NSUB, k % NSUB)
            return carry
        jax.lax.fori_loop(0, NG, pre_body, 0)

    mfill_s[...] = _fill(lambda i: jnp.where(i < 2 * M, i // M, (i - 2 * M) // SEG),
                         lambda i: jnp.where(i < 2 * M, i % M, M + (i - 2 * M) % SEG), RA)
    cm.wait()
    x2a_s[...] = jnp.zeros_like(x2a_s)
    x2_s[...] = jnp.zeros_like(x2_s)
    x1a_s[...] = jnp.zeros_like(x1a_s)
    m0 = mem0_s[...]
    _store_tiles(ha_s, 0, jnp.concatenate([m0, m0], axis=0))
    _store_tiles(ha_s, 2 * M, _ln(xr_s[0].astype(F32)).astype(BF16))
    _store_tiles(ha_s, 2 * M + SEG, jnp.zeros((SEG, D), BF16))

    def attention_phase(ha, fill, filler, pre_idx=None):
        allowed = fill == 0.0
        rows = fill.shape[0]

        def qkv(h):
            q = _dot(ha, _unpack(wq_s[h]))
            kk = _dot(ha, _unpack(wk_s[h]))
            v = _dot(ha, _unpack(wv_s[h]))
            res = [(q * scale).astype(BF16), kk.astype(BF16), v.astype(BF16)]
            if pre_idx is not None:
                res = [jnp.concatenate([r[0:2 * M], _unpack(pre_s[pre_idx, w, h]), r[2 * M:]], axis=0)
                       for w, r in enumerate(res)]
            return res

        def probs(q, kk):
            s = jax.lax.dot_general(q, kk, (((1,), (1,)), ((), ())), preferred_element_type=F32)
            s = jnp.where(allowed, s, fill)
            p = jnp.exp(s - jnp.max(s, axis=-1, keepdims=True))
            return (p * _recip(jnp.sum(p, axis=-1, keepdims=True))).astype(BF16)

        qs, ps = {}, {}
        for i in range(H + 2):
            if i < H:
                qs[i] = qkv(i)
            else:
                filler(i - H)
            if 0 <= i - 1 < H:
                ps[i - 1] = probs(qs[i - 1][0], qs[i - 1][1])
            if 0 <= i - 2 < H:
                o = _dot(ps.pop(i - 2), qs.pop(i - 2)[2])
                o_s[i - 2, 0:rows // 2, :] = _pack(o.astype(BF16))

    def out_proj(rows):
        o = jnp.concatenate([_unpack(o_s[h, 0:rows // 2, :]) for h in range(H)], axis=1)
        return jnp.concatenate([_dot(o, _unpack(wo_s[n])) for n in range(KT)], axis=1)

    def glu_chunk(hb, j):
        rows = hb.shape[0]
        g = _dot(hb, _unpack(wg_s[j]))
        u = _dot(hb, _unpack(wu_s[j]))
        act_s[j, 0:rows // 2, :] = _pack((jax.nn.sigmoid(g) * u).astype(BF16))

    def glu_down(rows):
        act = jnp.concatenate([_unpack(act_s[j, 0:rows // 2, :]) for j in range(FT)], axis=1)
        return jnp.concatenate([_dot(act, _unpack(wd_s[n])) for n in range(KT)], axis=1)

    def xseg(seg):
        return xr_s[seg % XR].astype(F32)

    def full_step(t, use_pre):
        x1a = x1a_s[...]
        x2a = x2a_s[...]
        _store_tiles(hb_s, 0, _ln(x1a).astype(BF16))
        _store_tiles(hb_s, SEG, _ln(x2a).astype(BF16))
        if use_pre:
            ha = jnp.concatenate(
                [jnp.concatenate([_unpack(ha_s[k, 0:M, :]), _unpack(ha_s[k, M + SEG // 2:RA // 2, :])], axis=0)
                 for k in range(KT)], axis=1)
            pre_idx = jnp.clip(t - PRE0, 0, NPRE - 1)
        else:
            ha = _cat(ha_s, KT)
            pre_idx = None
        hb = _cat(hb_s, KT)

        def filler(i):
            glu_chunk(hb, 2 * i)
            glu_chunk(hb, 2 * i + 1)
        attention_phase(ha, mfill_s[...], filler, pre_idx)
        for j in range(4, FT):
            glu_chunk(hb, j)
        z = glu_down(RB)

        xin = xseg(jnp.minimum(t, NSEG - 1))
        x2_old = x2_s[...]
        x2_new = x1a + z[0:SEG]
        x2_s[...] = x2_new
        ost_s[t % 2] = (x2a + z[SEG:RB]).astype(BF16)
        n1 = _ln(xseg(jnp.minimum(t + 1, NSEG - 1))).astype(BF16)
        n2 = _ln(x2_new).astype(BF16)

        y = out_proj(RA)
        _store_tiles(ha_s, 0, y[0:2 * M].astype(BF16))
        _store_tiles(ha_s, 2 * M, n1)
        _store_tiles(ha_s, 2 * M + SEG, n2)
        x1a_s[...] = xin + y[2 * M:2 * M + SEG]
        x2a_s[...] = x2_old + y[2 * M + SEG:RA]

    RH = 2 * M + SEG

    def a_half(layer, hook=None):
        tok0 = M + (SEG // 2) * layer
        ha = jnp.concatenate(
            [jnp.concatenate([_unpack(ha_s[k, 0:M, :]), _unpack(ha_s[k, tok0:tok0 + SEG // 2, :])], axis=0)
             for k in range(KT)], axis=1)
        fill = _fill(lambda i: jnp.where(i < 2 * M, i // M, layer),
                     lambda i: jnp.where(i < 2 * M, i % M, M + i - 2 * M), RH)
        attention_phase(ha, fill, lambda i: None)
        if hook is not None:
            hook()
        return out_proj(RH)

    def head_step(t):
        xb_s[...] = x1a_s[...]

        def hook():
            @pl.when(t == 0)
            def _():
                c_wo.wait()
                conv_cols(sto, wo_s, H * DH, KT)
        y = a_half(0, hook)
        m0f = mem0_s[...].astype(F32)
        _store_tiles(ha_s, 0, jnp.concatenate([y[0:M], m0f], axis=0).astype(BF16))
        _store_tiles(ha_s, 2 * M, _ln(xseg(t + 1)).astype(BF16))
        x1a_s[...] = xseg(t) + y[2 * M:RH]

        @pl.when(t == 1)
        def _():
            c_wg.wait()
            conv_cols(stg, wg_s, D, FT)
            c_wu.wait()
            conv_cols(stu, wu_s, D, FT)
            c_wd.wait()
            conv_cols(std, wd_s, FF, KT)
            xb = xb_s[...]
            hb = _ln(xb).astype(BF16)
            for j in range(FT):
                glu_chunk(hb, j)
            res = xb + glu_down(SEG)
            x2_s[...] = res
            _store_tiles(ha_s, 2 * M + SEG, _ln(res).astype(BF16))

    def tail_step(t):
        first = t == NSEG
        xb_s[...] = jnp.where(first, x1a_s[...], x2a_s[...])
        y_old = x2a_s[...]
        y = a_half(1)
        _store_tiles(ha_s, 0, y[0:2 * M].astype(BF16))
        x2a_new = x2_s[...] + y[2 * M:RH]
        x2a_s[...] = x2a_new
        xin0 = xb_s[...]
        xin1 = jnp.where(first, y_old, x2a_new)
        hb = jnp.concatenate([_ln(xin0).astype(BF16), _ln(xin1).astype(BF16)], axis=0)
        for j in range(FT):
            glu_chunk(hb, j)
        z = glu_down(RB)
        res0 = xin0 + z[0:SEG]
        res1 = xin1 + z[SEG:RB]

        @pl.when(first)
        def _():
            x2_s[...] = res0
            _store_tiles(ha_s, 2 * M + SEG, _ln(res0).astype(BF16))
            out_copy(t - 2).wait()
            ost_s[0] = res1.astype(BF16)
            out_copy(t).start()

        @pl.when(jnp.logical_not(first))
        def _():
            out_copy(t - 2).wait()
            ost_s[1] = res0.astype(BF16)
            out_copy(t).start()
            out_copy(t - 1).wait()
            ost_s[0] = res1.astype(BF16)
            out_copy(t + 1).start()

    def x_next(t):
        seg = jnp.minimum(t, NSEG - 1)
        return pltpu.make_async_copy(x_hbm.at[pl.ds(pl.multiple_of(seg * SEG, SEG), SEG)],
                                     xr_s.at[t % XR], sem_x.at[t % XR])

    def head_body(t, carry):
        x_copy(t + XPF).start()
        head_step(t)
        return carry

    def pre_body_step(t, carry):
        @pl.when(t >= 5)
        def _():
            out_copy(t - 2).wait()

        @pl.when(t + 1 >= PRE0 + NPRE)
        def _():
            x_copy(t + 1).wait()
        x_copy(t + XPF).start()
        full_step(t, True)

        @pl.when(t >= 3)
        def _():
            out_copy(t).start()
        return carry

    def full_body(t, carry):
        out_copy(t - 2).wait()
        x_next(t + 1).wait()
        x_next(t + XPF).start()
        full_step(t, False)
        out_copy(t).start()
        return carry

    def tail_body(t, carry):
        tail_step(t)
        return carry

    jax.lax.fori_loop(0, 2, head_body, 0)
    jax.lax.fori_loop(PRE0, PRE0 + NPRE, pre_body_step, 0)
    jax.lax.fori_loop(PRE0 + NPRE, NSEG, full_body, 0)
    jax.lax.fori_loop(NSEG, NSEG + 2, tail_body, 0)
    for s in range(NSEG + 1, NSEG + XPF):
        x_next(s).wait()
    out_copy(NSTEP - 2).wait()
    out_copy(NSTEP - 1).wait()


@jax.jit
def pallas_interleave_layers__memory_aug_recurrent_mem_tr__glu_gated_glu__prompt_kernel(A_x, A_mem0, A_Wq, A_Wk, A_Wv, A_Wo, A_seg_len, B_x, B_w_gate, B_w_up, B_w_down):
    x = A_x.reshape(S, D)
    mem0 = A_mem0.reshape(M, D)
    wo = A_Wo.reshape(H * DH, D)
    any_spec = pl.BlockSpec(memory_space=pl.ANY)
    out = pl.pallas_call(
        _kernel,
        out_shape=jax.ShapeDtypeStruct((S, D), BF16),
        in_specs=[any_spec] * 9,
        out_specs=any_spec,
        scratch_shapes=[
            pltpu.VMEM((XR, SEG, D), BF16),
            pltpu.VMEM((M, D), BF16),
            pltpu.VMEM((H, D // 2, DH), U32),
            pltpu.VMEM((H, D // 2, DH), U32),
            pltpu.VMEM((H, D // 2, DH), U32),
            pltpu.VMEM((KT, H * DH // 2, 128), U32),
            pltpu.VMEM((FT, D // 2, 128), U32),
            pltpu.VMEM((FT, D // 2, 128), U32),
            pltpu.VMEM((KT, FF // 2, 128), U32),
            pltpu.VMEM((2 * NCH, DCH, H, DH), BF16),
            pltpu.VMEM((H * DH, D), BF16),
            pltpu.VMEM((D, FF), BF16),
            pltpu.VMEM((D, FF), BF16),
            pltpu.VMEM((FF, D), BF16),
            pltpu.VMEM((KT, RA // 2, 128), U32),
            pltpu.VMEM((KT, RB // 2, 128), U32),
            pltpu.VMEM((KT, NPRE * SEG // 2, 128), U32),
            pltpu.VMEM((NPRE, 3, H, SEG // 2, 128), U32),
            pltpu.VMEM((H, RA // 2, 128), U32),
            pltpu.VMEM((FT, RB // 2, 128), U32),
            pltpu.VMEM((SEG, D), F32),
            pltpu.VMEM((SEG, D), F32),
            pltpu.VMEM((SEG, D), F32),
            pltpu.VMEM((SEG, D), F32),
            pltpu.VMEM((2, SEG, D), BF16),
            pltpu.VMEM((RA, RA), F32),
            pltpu.SemaphoreType.DMA((XR,)),
            pltpu.SemaphoreType.DMA,
            pltpu.SemaphoreType.DMA((2 * NCH,)),
            pltpu.SemaphoreType.DMA((4,)),
            pltpu.SemaphoreType.DMA((2,)),
        ],
        compiler_params=pltpu.CompilerParams(vmem_limit_bytes=120 * 1024 * 1024, disable_bounds_checks=True, disable_semaphore_checks=True),
    )(x, mem0, A_Wq, A_Wk, A_Wv, wo, B_w_gate, B_w_up, B_w_down)
    return out.reshape(1, S, D)
```

```python
import functools
import jax
import jax.numpy as jnp
import jax.experimental.pallas as pl
import jax.experimental.pallas.tpu as pltpu

F32 = jnp.float32
BF16 = jnp.bfloat16
U32 = jnp.uint32

S, D, H, DH, M, SEG, FF = 2048, 1024, 32, 128, 8, 32, 3584
NSEG = S // SEG
KT = D // 128
FT = FF // 128
RA = 2 * M + 2 * SEG
RB = 2 * SEG
NSTEP = NSEG + 3
DCH = 128
NCH = D // DCH
NPRE = 9
PRE0 = 2
XR = 16
XPF = 12
HG = 8
EPS = 1e-5
NEG_REF = -1e9


def _ln(x):
    m = jnp.mean(x, axis=-1, keepdims=True)
    xc = x - m
    v = jnp.mean(xc * xc, axis=-1, keepdims=True)
    return xc * jax.lax.rsqrt(v + EPS)


def _pack(x):
    return pltpu.bitcast(x, U32)


def _unpack(x):
    return pltpu.bitcast(x, BF16)


def _cat(ref, n):
    return jnp.concatenate([_unpack(ref[k]) for k in range(n)], axis=1)


def _store_tiles(ref, r0, x):
    rows = x.shape[0]
    for k in range(KT):
        ref[k, r0 // 2:(r0 + rows) // 2, :] = _pack(x[:, k * 128:(k + 1) * 128])


def _recip(x):
    r = pl.reciprocal(x, approx=True)
    return r * (2.0 - x * r)


def _dot(a, b):
    return jnp.dot(a, b, preferred_element_type=F32)


def _fill(rows_layer, rows_pos, n):
    r = jax.lax.broadcasted_iota(jnp.int32, (n, n), 0)
    c = jax.lax.broadcasted_iota(jnp.int32, (n, n), 1)
    same = rows_layer(r) == rows_layer(c)
    ok = (rows_pos(r) < M) | (rows_pos(r) >= rows_pos(c))
    return jnp.where(same, jnp.where(ok, 0.0, NEG_REF), -jnp.inf).astype(F32)


def _kernel(x_hbm, mem0_hbm, wq_hbm, wk_hbm, wv_hbm, wo_hbm, wg_hbm, wu_hbm, wd_hbm,
            out_hbm,
            xr_s, mem0_s, wq_s, wk_s, wv_s, wo_s, wg_s, wu_s, wd_s,
            st3, sto, stg, stu, std,
            ha_s, hb_s, hp_s, pre_s, acc_s, o_s, act_s, x1a_s, x2_s, x2a_s, xb_s, ost_s, mfill_s,
            sem_x, sem_m, sem_st, sem_w, sem_o):
    scale = DH ** -0.5

    def x_copy(seg):
        return pltpu.make_async_copy(x_hbm.at[pl.ds(pl.multiple_of(seg * SEG, SEG), SEG)],
                                     xr_s.at[seg % XR], sem_x.at[seg % XR])

    def out_copy(t):
        seg = t - 3
        return pltpu.make_async_copy(ost_s.at[t % 2],
                                     out_hbm.at[pl.ds(pl.multiple_of(seg * SEG, SEG), SEG)], sem_o.at[t % 2])

    NQ = H // HG

    def c_wo(q):
        n = H * DH // NQ
        r = pl.ds(pl.multiple_of(q * n, n), n)
        return pltpu.make_async_copy(wo_hbm.at[r], sto.at[r], sem_w.at[3 + q])
    c_wg = pltpu.make_async_copy(wg_hbm, stg, sem_w.at[0])
    c_wu = pltpu.make_async_copy(wu_hbm, stu, sem_w.at[1])
    c_wd = pltpu.make_async_copy(wd_hbm, std, sem_w.at[2])

    def conv_cols(src, dst, nrows, ntile):
        def body(c, carry):
            blk = src[pl.ds(pl.multiple_of(c * DCH, DCH), DCH), :]
            rows = pl.ds(pl.multiple_of(c * (DCH // 2), DCH // 2), DCH // 2)
            for j in range(ntile):
                dst[j, rows, :] = _pack(blk[:, j * 128:(j + 1) * 128])
            return carry
        jax.lax.fori_loop(0, nrows // DCH, body, 0)

    cm = pltpu.make_async_copy(mem0_hbm, mem0_s, sem_m)
    cm.start()
    for s in range(XPF):
        x_copy(s).start()

    qkv_src = [wq_hbm, wk_hbm, wv_hbm]
    qkv_dst = [wq_s, wk_s, wv_s]

    def st_copy(w, c):
        slot = (w % 2) * NCH + c
        return pltpu.make_async_copy(qkv_src[w].at[pl.ds(pl.multiple_of(c * DCH, DCH), DCH)], st3.at[slot], sem_st.at[slot])

    SUB = 16
    NSUB = DCH // SUB

    def convert_sub(w, c, s):
        x = pltpu.bitcast(st3[(w % 2) * NCH + c, s * SUB:(s + 1) * SUB], U32)
        x = x.reshape(SUB // 2, 2, H // 2, DH)
        a, b = x[:, 0], x[:, 1]
        lo = jnp.swapaxes((a & jnp.uint32(0xFFFF)) | (b << 16), 0, 1)
        hi = jnp.swapaxes((a >> 16) | (b & jnp.uint32(0xFFFF0000)), 0, 1)
        rows = pl.ds(pl.multiple_of(c * (DCH // 2) + s * (SUB // 2), SUB // 2), SUB // 2)
        for i in range(H // 2):
            qkv_dst[w][2 * i, rows, :] = lo[i]
            qkv_dst[w][2 * i + 1, rows, :] = hi[i]

    def convert(w, c):
        for s in range(NSUB):
            convert_sub(w, c, s)

    LOOK = 5
    for c in range(LOOK):
        st_copy(0, c).start()
    for s in range(PRE0 + NPRE):
        x_copy(s).wait()
    for s in range(NPRE):
        _store_tiles(hp_s, s * SEG, _ln(xr_s[PRE0 + s].astype(F32)).astype(BF16))

    def store_pre(w, h, r):
        r = _pack(r.astype(BF16))
        for s in range(NPRE):
            pre_s[s, w, h] = r[s * (SEG // 2):(s + 1) * (SEG // 2)]

    order = [(g // NCH, g % NCH) for g in range(LOOK, 3 * NCH)]
    HPC = H // NCH

    def start_wo():
        for q in range(NQ):
            c_wo(q).start()
    hooks = {(1, 3): start_wo, (1, 7): c_wg.start, (2, 3): c_wu.start, (2, 6): c_wd.start}

    def finish(w, c):
        for j in range(HPC):
            h = c * HPC + j
            r = acc_s[w % 2, h]
            store_pre(w, h, r * scale if w == 0 else r)

    for w in range(3):
        def w_body(c, carry, w=w):
            if w == 0:
                for cc in range(NCH):
                    @pl.when(c == cc)
                    def _(cc=cc):
                        st_copy(*order[2 * cc]).start()
                        st_copy(*order[2 * cc + 1]).start()
            for (hw, hc), fn in hooks.items():
                if hw == w:
                    pl.when(c == hc)(fn)
            st_copy(w, c).wait()
            convert(w, c)
            hpc = _unpack(hp_s[c])
            rows = pl.ds(pl.multiple_of(c * (DCH // 2), DCH // 2), DCH // 2)
            for h in range(H):
                part = _dot(hpc, _unpack(qkv_dst[w][h, rows, :]))
                acc_s[w % 2, h] = jnp.where(c > 0, acc_s[w % 2, h], 0.0) + part
            if w > 0:
                finish(w - 1, c)
            return carry
        jax.lax.fori_loop(0, NCH, w_body, 0)
        if w == 0:
            for wc in order[2 * NCH:]:
                st_copy(*wc).start()

    def v_body(c, carry):
        @pl.when(c % (NCH // NQ) == 0)
        def _():
            c_wo(c // (NCH // NQ)).wait()
        finish(2, c)
        for i in range(H // NCH):
            cc = c * (H // NCH) + i
            blk = sto[pl.ds(pl.multiple_of(cc * DCH, DCH), DCH), :]
            rows = pl.ds(pl.multiple_of(cc * (DCH // 2), DCH // 2), DCH // 2)
            for n in range(KT):
                wo_s[n, rows, :] = _pack(blk[:, n * 128:(n + 1) * 128])
        return carry
    jax.lax.fori_loop(0, NCH, v_body, 0)

    mfill_s[...] = _fill(lambda i: jnp.where(i < 2 * M, i // M, (i - 2 * M) // SEG),
                         lambda i: jnp.where(i < 2 * M, i % M, M + (i - 2 * M) % SEG), RA)
    cm.wait()
    x2a_s[...] = jnp.zeros_like(x2a_s)
    x2_s[...] = jnp.zeros_like(x2_s)
    x1a_s[...] = jnp.zeros_like(x1a_s)
    m0 = mem0_s[...]
    _store_tiles(ha_s, 0, jnp.concatenate([m0, m0], axis=0))
    _store_tiles(ha_s, 2 * M, _ln(xr_s[0].astype(F32)).astype(BF16))
    _store_tiles(ha_s, 2 * M + SEG, jnp.zeros((SEG, D), BF16))

    def attention_phase(ha, fill, filler, pre_idx=None):
        allowed = fill == 0.0
        rows = fill.shape[0]

        def qkv(h):
            q = _dot(ha, _unpack(wq_s[h]))
            kk = _dot(ha, _unpack(wk_s[h]))
            v = _dot(ha, _unpack(wv_s[h]))
            res = [(q * scale).astype(BF16), kk.astype(BF16), v.astype(BF16)]
            if pre_idx is not None:
                res = [jnp.concatenate([r[0:2 * M], _unpack(pre_s[pre_idx, w, h]), r[2 * M:]], axis=0)
                       for w, r in enumerate(res)]
            return res

        def probs(q, kk):
            s = jax.lax.dot_general(q, kk, (((1,), (1,)), ((), ())), preferred_element_type=F32)
            s = jnp.where(allowed, s, fill)
            p = jnp.exp(s - jnp.max(s, axis=-1, keepdims=True))
            return (p * _recip(jnp.sum(p, axis=-1, keepdims=True))).astype(BF16)

        qs, ps = {}, {}
        for i in range(H + 2):
            if i < H:
                qs[i] = qkv(i)
            else:
                filler(i - H)
            if 0 <= i - 1 < H:
                ps[i - 1] = probs(qs[i - 1][0], qs[i - 1][1])
            if 0 <= i - 2 < H:
                o = _dot(ps.pop(i - 2), qs.pop(i - 2)[2])
                o_s[i - 2, 0:rows // 2, :] = _pack(o.astype(BF16))

    def out_proj(rows):
        o = jnp.concatenate([_unpack(o_s[h, 0:rows // 2, :]) for h in range(H)], axis=1)
        return jnp.concatenate([_dot(o, _unpack(wo_s[n])) for n in range(KT)], axis=1)

    def glu_chunk(hb, j):
        rows = hb.shape[0]
        g = _dot(hb, _unpack(wg_s[j]))
        u = _dot(hb, _unpack(wu_s[j]))
        act_s[j, 0:rows // 2, :] = _pack((jax.nn.sigmoid(g) * u).astype(BF16))

    def glu_down(rows):
        act = jnp.concatenate([_unpack(act_s[j, 0:rows // 2, :]) for j in range(FT)], axis=1)
        return jnp.concatenate([_dot(act, _unpack(wd_s[n])) for n in range(KT)], axis=1)

    def xseg(seg):
        return xr_s[seg % XR].astype(F32)

    def full_step(t, use_pre):
        x1a = x1a_s[...]
        x2a = x2a_s[...]
        _store_tiles(hb_s, 0, _ln(x1a).astype(BF16))
        _store_tiles(hb_s, SEG, _ln(x2a).astype(BF16))
        if use_pre:
            ha = jnp.concatenate(
                [jnp.concatenate([_unpack(ha_s[k, 0:M, :]), _unpack(ha_s[k, M + SEG // 2:RA // 2, :])], axis=0)
                 for k in range(KT)], axis=1)
            pre_idx = jnp.clip(t - PRE0, 0, NPRE - 1)
        else:
            ha = _cat(ha_s, KT)
            pre_idx = None
        hb = _cat(hb_s, KT)

        def filler(i):
            glu_chunk(hb, 2 * i)
            glu_chunk(hb, 2 * i + 1)
        attention_phase(ha, mfill_s[...], filler, pre_idx)
        for j in range(4, FT):
            glu_chunk(hb, j)
        z = glu_down(RB)

        xin = xseg(jnp.minimum(t, NSEG - 1))
        x2_old = x2_s[...]
        x2_new = x1a + z[0:SEG]
        x2_s[...] = x2_new
        ost_s[t % 2] = (x2a + z[SEG:RB]).astype(BF16)
        n1 = _ln(xseg(jnp.minimum(t + 1, NSEG - 1))).astype(BF16)
        n2 = _ln(x2_new).astype(BF16)

        y = out_proj(RA)
        _store_tiles(ha_s, 0, y[0:2 * M].astype(BF16))
        _store_tiles(ha_s, 2 * M, n1)
        _store_tiles(ha_s, 2 * M + SEG, n2)
        x1a_s[...] = xin + y[2 * M:2 * M + SEG]
        x2a_s[...] = x2_old + y[2 * M + SEG:RA]

    RH = 2 * M + SEG

    def a_half(layer, hook=None):
        tok0 = M + (SEG // 2) * layer
        ha = jnp.concatenate(
            [jnp.concatenate([_unpack(ha_s[k, 0:M, :]), _unpack(ha_s[k, tok0:tok0 + SEG // 2, :])], axis=0)
             for k in range(KT)], axis=1)
        fill = _fill(lambda i: jnp.where(i < 2 * M, i // M, layer),
                     lambda i: jnp.where(i < 2 * M, i % M, M + i - 2 * M), RH)
        attention_phase(ha, fill, lambda i: None)
        if hook is not None:
            hook()
        return out_proj(RH)

    def head_step(t):
        xb_s[...] = x1a_s[...]

        y = a_half(0)
        m0f = mem0_s[...].astype(F32)
        _store_tiles(ha_s, 0, jnp.concatenate([y[0:M], m0f], axis=0).astype(BF16))
        _store_tiles(ha_s, 2 * M, _ln(xseg(t + 1)).astype(BF16))
        x1a_s[...] = xseg(t) + y[2 * M:RH]

        @pl.when(t == 1)
        def _():
            c_wg.wait()
            conv_cols(stg, wg_s, D, FT)
            c_wu.wait()
            conv_cols(stu, wu_s, D, FT)
            c_wd.wait()
            conv_cols(std, wd_s, FF, KT)
            xb = xb_s[...]
            hb = _ln(xb).astype(BF16)
            for j in range(FT):
                glu_chunk(hb, j)
            res = xb + glu_down(SEG)
            x2_s[...] = res
            _store_tiles(ha_s, 2 * M + SEG, _ln(res).astype(BF16))

    def tail_step(t):
        first = t == NSEG
        xb_s[...] = jnp.where(first, x1a_s[...], x2a_s[...])
        y_old = x2a_s[...]
        y = a_half(1)
        _store_tiles(ha_s, 0, y[0:2 * M].astype(BF16))
        x2a_new = x2_s[...] + y[2 * M:RH]
        x2a_s[...] = x2a_new
        xin0 = xb_s[...]
        xin1 = jnp.where(first, y_old, x2a_new)
        hb = jnp.concatenate([_ln(xin0).astype(BF16), _ln(xin1).astype(BF16)], axis=0)
        for j in range(FT):
            glu_chunk(hb, j)
        z = glu_down(RB)
        res0 = xin0 + z[0:SEG]
        res1 = xin1 + z[SEG:RB]

        @pl.when(first)
        def _():
            x2_s[...] = res0
            _store_tiles(ha_s, 2 * M + SEG, _ln(res0).astype(BF16))
            out_copy(t - 2).wait()
            ost_s[0] = res1.astype(BF16)
            out_copy(t).start()

        @pl.when(jnp.logical_not(first))
        def _():
            out_copy(t - 2).wait()
            ost_s[1] = res0.astype(BF16)
            out_copy(t).start()
            out_copy(t - 1).wait()
            ost_s[0] = res1.astype(BF16)
            out_copy(t + 1).start()

    def x_next(t):
        seg = jnp.minimum(t, NSEG - 1)
        return pltpu.make_async_copy(x_hbm.at[pl.ds(pl.multiple_of(seg * SEG, SEG), SEG)],
                                     xr_s.at[t % XR], sem_x.at[t % XR])

    def head_body(t, carry):
        x_copy(t + XPF).start()
        head_step(t)
        return carry

    def pre_body_step(t, carry):
        @pl.when(t >= 5)
        def _():
            out_copy(t - 2).wait()

        @pl.when(t + 1 >= PRE0 + NPRE)
        def _():
            x_copy(t + 1).wait()
        x_copy(t + XPF).start()
        full_step(t, True)

        @pl.when(t >= 3)
        def _():
            out_copy(t).start()
        return carry

    def full_body(t, carry):
        out_copy(t - 2).wait()
        x_next(t + 1).wait()
        x_next(t + XPF).start()
        full_step(t, False)
        out_copy(t).start()
        return carry

    def tail_body(t, carry):
        tail_step(t)
        return carry

    jax.lax.fori_loop(0, 2, head_body, 0)
    jax.lax.fori_loop(PRE0, PRE0 + NPRE, pre_body_step, 0)
    jax.lax.fori_loop(PRE0 + NPRE, NSEG, full_body, 0)
    jax.lax.fori_loop(NSEG, NSEG + 2, tail_body, 0)
    for s in range(NSEG + 1, NSEG + XPF):
        x_next(s).wait()
    out_copy(NSTEP - 2).wait()
    out_copy(NSTEP - 1).wait()


@jax.jit
def pallas_interleave_layers__memory_aug_recurrent_mem_tr__glu_gated_glu__prompt_kernel(A_x, A_mem0, A_Wq, A_Wk, A_Wv, A_Wo, A_seg_len, B_x, B_w_gate, B_w_up, B_w_down):
    x = A_x.reshape(S, D)
    mem0 = A_mem0.reshape(M, D)
    wo = A_Wo.reshape(H * DH, D)
    any_spec = pl.BlockSpec(memory_space=pl.ANY)
    out = pl.pallas_call(
        _kernel,
        out_shape=jax.ShapeDtypeStruct((S, D), BF16),
        in_specs=[any_spec] * 9,
        out_specs=any_spec,
        scratch_shapes=[
            pltpu.VMEM((XR, SEG, D), BF16),
            pltpu.VMEM((M, D), BF16),
            pltpu.VMEM((H, D // 2, DH), U32),
            pltpu.VMEM((H, D // 2, DH), U32),
            pltpu.VMEM((H, D // 2, DH), U32),
            pltpu.VMEM((KT, H * DH // 2, 128), U32),
            pltpu.VMEM((FT, D // 2, 128), U32),
            pltpu.VMEM((FT, D // 2, 128), U32),
            pltpu.VMEM((KT, FF // 2, 128), U32),
            pltpu.VMEM((2 * NCH, DCH, H, DH), BF16),
            pltpu.VMEM((H * DH, D), BF16),
            pltpu.VMEM((D, FF), BF16),
            pltpu.VMEM((D, FF), BF16),
            pltpu.VMEM((FF, D), BF16),
            pltpu.VMEM((KT, RA // 2, 128), U32),
            pltpu.VMEM((KT, RB // 2, 128), U32),
            pltpu.VMEM((KT, NPRE * SEG // 2, 128), U32),
            pltpu.VMEM((NPRE, 3, H, SEG // 2, 128), U32),
            pltpu.VMEM((2, H, NPRE * SEG, DH), F32),
            pltpu.VMEM((H, RA // 2, 128), U32),
            pltpu.VMEM((FT, RB // 2, 128), U32),
            pltpu.VMEM((SEG, D), F32),
            pltpu.VMEM((SEG, D), F32),
            pltpu.VMEM((SEG, D), F32),
            pltpu.VMEM((SEG, D), F32),
            pltpu.VMEM((2, SEG, D), BF16),
            pltpu.VMEM((RA, RA), F32),
            pltpu.SemaphoreType.DMA((XR,)),
            pltpu.SemaphoreType.DMA,
            pltpu.SemaphoreType.DMA((2 * NCH,)),
            pltpu.SemaphoreType.DMA((3 + H // HG,)),
            pltpu.SemaphoreType.DMA((2,)),
        ],
        compiler_params=pltpu.CompilerParams(vmem_limit_bytes=120 * 1024 * 1024, disable_bounds_checks=True, disable_semaphore_checks=True),
    )(x, mem0, A_Wq, A_Wk, A_Wv, wo, B_w_gate, B_w_up, B_w_down)
    return out.reshape(1, S, D)
```

```python
import jax
import jax.numpy as jnp
import jax.experimental.pallas as pl
import jax.experimental.pallas.tpu as pltpu

F32 = jnp.float32
BF16 = jnp.bfloat16
U32 = jnp.uint32

S, D, H, DH, M, SEG, FF = 2048, 1024, 32, 128, 8, 32, 3584
NSEG = S // SEG
KT = D // 128
FT = FF // 128
RA = 2 * M + 2 * SEG
RB = 2 * SEG
NSTEP = NSEG + 3
DCH = 128
NCH = D // DCH
NPRE = 10
PRE0 = 2
XR = 16
XPF = 13
NQ = 4
EPS = 1e-5
NEG_REF = -1e9


def _ln(x):
    m = jnp.mean(x, axis=-1, keepdims=True)
    xc = x - m
    v = jnp.mean(xc * xc, axis=-1, keepdims=True)
    return xc * jax.lax.rsqrt(v + EPS)


def _pack(x):
    return pltpu.bitcast(x, U32)


def _unpack(x):
    return pltpu.bitcast(x, BF16)


def _cat(ref, n):
    return jnp.concatenate([_unpack(ref[k]) for k in range(n)], axis=1)


def _store_tiles(ref, r0, x):
    rows = x.shape[0]
    for k in range(KT):
        ref[k, r0 // 2:(r0 + rows) // 2, :] = _pack(x[:, k * 128:(k + 1) * 128])


def _recip(x):
    r = pl.reciprocal(x, approx=True)
    return r * (2.0 - x * r)


def _dot(a, b):
    return jnp.dot(a, b, preferred_element_type=F32)


def _fill(rows_layer, rows_pos, n):
    r = jax.lax.broadcasted_iota(jnp.int32, (n, n), 0)
    c = jax.lax.broadcasted_iota(jnp.int32, (n, n), 1)
    same = rows_layer(r) == rows_layer(c)
    ok = (rows_pos(r) < M) | (rows_pos(r) >= rows_pos(c))
    return jnp.where(same, jnp.where(ok, 0.0, NEG_REF), -jnp.inf).astype(F32)


def _kernel(x_hbm, mem0_hbm, wq_hbm, wk_hbm, wv_hbm, wo_hbm, wg_hbm, wu_hbm, wd_hbm,
            out_hbm,
            xr_s, mem0_s, wq_s, wk_s, wv_s, wo_s, wg_s, wu_s, wd_s,
            st3, sto, stg, stu, std,
            ha_s, hb_s, hp_s, pre_s, acc_s, o_s, act_s, x1a_s, x2_s, x2a_s, xb_s, ost_s, mfill_s,
            sem_x, sem_m, sem_st, sem_w, sem_o):
    scale = DH ** -0.5

    def x_copy(seg):
        return pltpu.make_async_copy(x_hbm.at[pl.ds(pl.multiple_of(seg * SEG, SEG), SEG)],
                                     xr_s.at[seg & (XR - 1)], sem_x.at[seg & (XR - 1)])

    def out_copy(t):
        seg = t - 3
        return pltpu.make_async_copy(ost_s.at[t & 1],
                                     out_hbm.at[pl.ds(pl.multiple_of(seg * SEG, SEG), SEG)], sem_o.at[t & 1])

    def c_wo(q):
        n = H * DH // NQ
        r = pl.ds(pl.multiple_of(q * n, n), n)
        return pltpu.make_async_copy(wo_hbm.at[r], sto.at[r], sem_w.at[3 + q])
    c_wg = pltpu.make_async_copy(wg_hbm, stg, sem_w.at[0])
    c_wu = pltpu.make_async_copy(wu_hbm, stu, sem_w.at[1])
    c_wd = pltpu.make_async_copy(wd_hbm, std, sem_w.at[2])

    def conv_cols(src, dst, nrows, ntile):
        def body(c, carry):
            blk = src[pl.ds(pl.multiple_of(c * DCH, DCH), DCH), :]
            rows = pl.ds(pl.multiple_of(c * (DCH // 2), DCH // 2), DCH // 2)
            for j in range(ntile):
                dst[j, rows, :] = _pack(blk[:, j * 128:(j + 1) * 128])
            return carry
        jax.lax.fori_loop(0, nrows // DCH, body, 0)

    cm = pltpu.make_async_copy(mem0_hbm, mem0_s, sem_m)
    cm.start()
    for s in range(XPF):
        x_copy(s).start()

    qkv_src = [wq_hbm, wk_hbm, wv_hbm]
    qkv_dst = [wq_s, wk_s, wv_s]

    def st_copy(w, c):
        slot = (w % 2) * NCH + c
        return pltpu.make_async_copy(qkv_src[w].at[pl.ds(pl.multiple_of(c * DCH, DCH), DCH)], st3.at[slot], sem_st.at[slot])

    SUB = 16
    NSUB = DCH // SUB

    def convert_sub(w, c, s):
        x = pltpu.bitcast(st3[(w % 2) * NCH + c, s * SUB:(s + 1) * SUB], U32)
        x = x.reshape(SUB // 2, 2, H // 2, DH)
        a, b = x[:, 0], x[:, 1]
        lo = jnp.swapaxes((a & jnp.uint32(0xFFFF)) | (b << 16), 0, 1)
        hi = jnp.swapaxes((a >> 16) | (b & jnp.uint32(0xFFFF0000)), 0, 1)
        rows = pl.ds(pl.multiple_of(c * (DCH // 2) + s * (SUB // 2), SUB // 2), SUB // 2)
        for i in range(H // 2):
            qkv_dst[w][2 * i, rows, :] = lo[i]
            qkv_dst[w][2 * i + 1, rows, :] = hi[i]

    def convert(w, c):
        for s in range(NSUB):
            convert_sub(w, c, s)

    LOOK = 5
    for c in range(LOOK):
        st_copy(0, c).start()
    for s in range(PRE0 + NPRE):
        x_copy(s).wait()
    for s in range(NPRE):
        _store_tiles(hp_s, s * SEG, _ln(xr_s[PRE0 + s].astype(F32)).astype(BF16))

    def store_pre(w, h, r):
        r = _pack(r.astype(BF16))
        for s in range(NPRE):
            pre_s[s, w, h] = r[s * (SEG // 2):(s + 1) * (SEG // 2)]

    order = [(g // NCH, g % NCH) for g in range(LOOK, 3 * NCH)]
    HPC = H // NCH

    def start_wo():
        for q in range(NQ):
            c_wo(q).start()
    hooks = {(1, 3): start_wo, (1, 7): c_wg.start, (2, 3): c_wu.start, (2, 6): c_wd.start}

    def finish(w, c):
        for j in range(HPC):
            h = c * HPC + j
            r = acc_s[w % 2, h]
            store_pre(w, h, r * scale if w == 0 else r)

    for w in range(3):
        def w_body(c, carry, w=w):
            if w == 0:
                for cc in range(NCH):
                    @pl.when(c == cc)
                    def _(cc=cc):
                        st_copy(*order[2 * cc]).start()
                        st_copy(*order[2 * cc + 1]).start()
            for (hw, hc), fn in hooks.items():
                if hw == w:
                    pl.when(c == hc)(fn)
            st_copy(w, c).wait()
            convert(w, c)
            hpc = _unpack(hp_s[c])
            rows = pl.ds(pl.multiple_of(c * (DCH // 2), DCH // 2), DCH // 2)
            for h in range(H):
                part = _dot(hpc, _unpack(qkv_dst[w][h, rows, :]))
                acc_s[w % 2, h] = jnp.where(c > 0, acc_s[w % 2, h], 0.0) + part
            if w > 0:
                finish(w - 1, c)
            return carry
        jax.lax.fori_loop(0, NCH, w_body, 0)
        if w == 0:
            for wc in order[2 * NCH:]:
                st_copy(*wc).start()

    def v_body(c, carry):
        @pl.when(c % (NCH // NQ) == 0)
        def _():
            c_wo(c // (NCH // NQ)).wait()
        finish(2, c)
        for i in range(H // NCH):
            cc = c * (H // NCH) + i
            blk = sto[pl.ds(pl.multiple_of(cc * DCH, DCH), DCH), :]
            rows = pl.ds(pl.multiple_of(cc * (DCH // 2), DCH // 2), DCH // 2)
            for n in range(KT):
                wo_s[n, rows, :] = _pack(blk[:, n * 128:(n + 1) * 128])
        return carry
    jax.lax.fori_loop(0, NCH, v_body, 0)

    mfill_s[...] = _fill(lambda i: jnp.where(i < 2 * M, i // M, (i - 2 * M) // SEG),
                         lambda i: jnp.where(i < 2 * M, i % M, M + (i - 2 * M) % SEG), RA)
    cm.wait()
    x2a_s[...] = jnp.zeros_like(x2a_s)
    x2_s[...] = jnp.zeros_like(x2_s)
    x1a_s[...] = jnp.zeros_like(x1a_s)
    m0 = mem0_s[...]
    _store_tiles(ha_s, 0, jnp.concatenate([m0, m0], axis=0))
    _store_tiles(ha_s, 2 * M, _ln(xr_s[0].astype(F32)).astype(BF16))
    _store_tiles(ha_s, 2 * M + SEG, jnp.zeros((SEG, D), BF16))

    def attention_phase(ha, fill, filler, pre_idx=None):
        allowed = fill == 0.0
        rows = fill.shape[0]

        def qkv(h):
            q = _dot(ha, _unpack(wq_s[h]))
            kk = _dot(ha, _unpack(wk_s[h]))
            v = _dot(ha, _unpack(wv_s[h]))
            res = [(q * scale).astype(BF16), kk.astype(BF16), v.astype(BF16)]
            if pre_idx is not None:
                res = [jnp.concatenate([r[0:2 * M], _unpack(pre_s[pre_idx, w, h]), r[2 * M:]], axis=0)
                       for w, r in enumerate(res)]
            return res

        def probs(q, kk):
            s = jax.lax.dot_general(q, kk, (((1,), (1,)), ((), ())), preferred_element_type=F32)
            s = jnp.where(allowed, s, fill)
            p = jnp.exp(s - jnp.max(s, axis=-1, keepdims=True))
            return (p * _recip(jnp.sum(p, axis=-1, keepdims=True))).astype(BF16)

        qs, ps = {}, {}
        lag = 2 if ha.shape[0] == RA else 3
        for i in range(H + lag):
            if i < H:
                qs[i] = qkv(i)
            else:
                filler(i - H)
            if 0 <= i - 1 < H:
                ps[i - 1] = probs(qs[i - 1][0], qs[i - 1][1])
            if 0 <= i - lag < H:
                o = _dot(ps.pop(i - lag), qs.pop(i - lag)[2])
                o_s[i - lag, 0:rows // 2, :] = _pack(o.astype(BF16))

    def out_proj(rows):
        o = jnp.concatenate([_unpack(o_s[h, 0:rows // 2, :]) for h in range(H)], axis=1)
        return jnp.concatenate([_dot(o, _unpack(wo_s[n])) for n in range(KT)], axis=1)

    def glu_chunk(hb, j):
        rows = hb.shape[0]
        g = _dot(hb, _unpack(wg_s[j]))
        u = _dot(hb, _unpack(wu_s[j]))
        act_s[j, 0:rows // 2, :] = _pack((jax.nn.sigmoid(g) * u).astype(BF16))

    def glu_down(rows):
        act = jnp.concatenate([_unpack(act_s[j, 0:rows // 2, :]) for j in range(FT)], axis=1)
        return jnp.concatenate([_dot(act, _unpack(wd_s[n])) for n in range(KT)], axis=1)

    def xseg(seg):
        return xr_s[seg & (XR - 1)].astype(F32)

    def full_step(t, use_pre):
        x1a = x1a_s[...]
        x2a = x2a_s[...]
        _store_tiles(hb_s, 0, _ln(x1a).astype(BF16))
        _store_tiles(hb_s, SEG, _ln(x2a).astype(BF16))
        if use_pre:
            ha = jnp.concatenate(
                [jnp.concatenate([_unpack(ha_s[k, 0:M, :]), _unpack(ha_s[k, M + SEG // 2:RA // 2, :])], axis=0)
                 for k in range(KT)], axis=1)
            pre_idx = jnp.clip(t - PRE0, 0, NPRE - 1)
        else:
            ha = _cat(ha_s, KT)
            pre_idx = None
        hb = _cat(hb_s, KT)

        def filler(i):
            glu_chunk(hb, 2 * i)
            glu_chunk(hb, 2 * i + 1)
        attention_phase(ha, mfill_s[...], filler, pre_idx)
        for j in range(6 if use_pre else 4, FT):
            glu_chunk(hb, j)
        z = glu_down(RB)

        xin = xseg(t)
        x2_old = x2_s[...]
        x2_new = x1a + z[0:SEG]
        x2_s[...] = x2_new
        ost_s[t & 1] = (x2a + z[SEG:RB]).astype(BF16)
        n1 = _ln(xseg(jnp.minimum(t + 1, NSEG - 1))).astype(BF16)
        n2 = _ln(x2_new).astype(BF16)

        y = out_proj(RA)
        _store_tiles(ha_s, 0, y[0:2 * M].astype(BF16))
        _store_tiles(ha_s, 2 * M, n1)
        _store_tiles(ha_s, 2 * M + SEG, n2)
        x1a_s[...] = xin + y[2 * M:2 * M + SEG]
        x2a_s[...] = x2_old + y[2 * M + SEG:RA]

    RH = 2 * M + SEG

    def a_half(layer):
        tok0 = M + (SEG // 2) * layer
        ha = jnp.concatenate(
            [jnp.concatenate([_unpack(ha_s[k, 0:M, :]), _unpack(ha_s[k, tok0:tok0 + SEG // 2, :])], axis=0)
             for k in range(KT)], axis=1)
        fill = _fill(lambda i: jnp.where(i < 2 * M, i // M, layer),
                     lambda i: jnp.where(i < 2 * M, i % M, M + i - 2 * M), RH)
        attention_phase(ha, fill, lambda i: None)
        return out_proj(RH)

    def head_step(t):
        xb_s[...] = x1a_s[...]
        y = a_half(0)
        m0f = mem0_s[...].astype(F32)
        _store_tiles(ha_s, 0, jnp.concatenate([y[0:M], m0f], axis=0).astype(BF16))
        _store_tiles(ha_s, 2 * M, _ln(xseg(t + 1)).astype(BF16))
        x1a_s[...] = xseg(t) + y[2 * M:RH]

        @pl.when(t == 1)
        def _():
            c_wg.wait()
            conv_cols(stg, wg_s, D, FT)
            c_wu.wait()
            conv_cols(stu, wu_s, D, FT)
            c_wd.wait()
            conv_cols(std, wd_s, FF, KT)
            xb = xb_s[...]
            hb = _ln(xb).astype(BF16)
            for j in range(FT):
                glu_chunk(hb, j)
            res = xb + glu_down(SEG)
            x2_s[...] = res
            _store_tiles(ha_s, 2 * M + SEG, _ln(res).astype(BF16))

    def tail_step(t):
        first = t == NSEG
        xb_s[...] = jnp.where(first, x1a_s[...], x2a_s[...])
        y_old = x2a_s[...]
        y = a_half(1)
        _store_tiles(ha_s, 0, y[0:2 * M].astype(BF16))
        x2a_new = x2_s[...] + y[2 * M:RH]
        x2a_s[...] = x2a_new
        xin0 = xb_s[...]
        xin1 = jnp.where(first, y_old, x2a_new)
        hb = jnp.concatenate([_ln(xin0).astype(BF16), _ln(xin1).astype(BF16)], axis=0)
        for j in range(FT):
            glu_chunk(hb, j)
        z = glu_down(RB)
        res0 = xin0 + z[0:SEG]
        res1 = xin1 + z[SEG:RB]

        @pl.when(first)
        def _():
            x2_s[...] = res0
            _store_tiles(ha_s, 2 * M + SEG, _ln(res0).astype(BF16))
            out_copy(t - 2).wait()
            ost_s[0] = res1.astype(BF16)
            out_copy(t).start()

        @pl.when(jnp.logical_not(first))
        def _():
            out_copy(t - 2).wait()
            ost_s[1] = res0.astype(BF16)
            out_copy(t).start()
            out_copy(t - 1).wait()
            ost_s[0] = res1.astype(BF16)
            out_copy(t + 1).start()

    def x_next(t):
        seg = jnp.minimum(t, NSEG - 1)
        return pltpu.make_async_copy(x_hbm.at[pl.ds(pl.multiple_of(seg * SEG, SEG), SEG)],
                                     xr_s.at[t & (XR - 1)], sem_x.at[t & (XR - 1)])

    def head_body(t, carry):
        x_copy(t + XPF).start()
        head_step(t)
        return carry

    def pre_body_step(t, carry):
        @pl.when(t >= 5)
        def _():
            out_copy(t - 2).wait()

        @pl.when(t + 1 >= PRE0 + NPRE)
        def _():
            x_copy(t + 1).wait()
        x_copy(t + XPF).start()
        full_step(t, True)

        @pl.when(t >= 3)
        def _():
            out_copy(t).start()
        return carry

    def full_body(t, carry):
        out_copy(t - 2).wait()
        x_next(t + 1).wait()
        x_next(t + XPF).start()
        full_step(t, False)
        out_copy(t).start()
        return carry

    def tail_body(t, carry):
        tail_step(t)
        return carry

    jax.lax.fori_loop(0, 2, head_body, 0)
    jax.lax.fori_loop(PRE0, PRE0 + NPRE, pre_body_step, 0)
    jax.lax.fori_loop(PRE0 + NPRE, NSEG, full_body, 0)
    jax.lax.fori_loop(NSEG, NSEG + 2, tail_body, 0)
    for s in range(NSEG + 1, NSEG + XPF):
        x_next(s).wait()
    out_copy(NSTEP - 2).wait()
    out_copy(NSTEP - 1).wait()


@jax.jit
def pallas_interleave_layers__memory_aug_recurrent_mem_tr__glu_gated_glu__prompt_kernel(A_x, A_mem0, A_Wq, A_Wk, A_Wv, A_Wo, A_seg_len, B_x, B_w_gate, B_w_up, B_w_down):
    x = A_x.reshape(S, D)
    mem0 = A_mem0.reshape(M, D)
    wo = A_Wo.reshape(H * DH, D)
    any_spec = pl.BlockSpec(memory_space=pl.ANY)
    out = pl.pallas_call(
        _kernel,
        out_shape=jax.ShapeDtypeStruct((S, D), BF16),
        in_specs=[any_spec] * 9,
        out_specs=any_spec,
        scratch_shapes=[
            pltpu.VMEM((XR, SEG, D), BF16),
            pltpu.VMEM((M, D), BF16),
            pltpu.VMEM((H, D // 2, DH), U32),
            pltpu.VMEM((H, D // 2, DH), U32),
            pltpu.VMEM((H, D // 2, DH), U32),
            pltpu.VMEM((KT, H * DH // 2, 128), U32),
            pltpu.VMEM((FT, D // 2, 128), U32),
            pltpu.VMEM((FT, D // 2, 128), U32),
            pltpu.VMEM((KT, FF // 2, 128), U32),
            pltpu.VMEM((2 * NCH, DCH, H, DH), BF16),
            pltpu.VMEM((H * DH, D), BF16),
            pltpu.VMEM((D, FF), BF16),
            pltpu.VMEM((D, FF), BF16),
            pltpu.VMEM((FF, D), BF16),
            pltpu.VMEM((KT, RA // 2, 128), U32),
            pltpu.VMEM((KT, RB // 2, 128), U32),
            pltpu.VMEM((KT, NPRE * SEG // 2, 128), U32),
            pltpu.VMEM((NPRE, 3, H, SEG // 2, 128), U32),
            pltpu.VMEM((2, H, NPRE * SEG, DH), F32),
            pltpu.VMEM((H, RA // 2, 128), U32),
            pltpu.VMEM((FT, RB // 2, 128), U32),
            pltpu.VMEM((SEG, D), F32),
            pltpu.VMEM((SEG, D), F32),
            pltpu.VMEM((SEG, D), F32),
            pltpu.VMEM((SEG, D), F32),
            pltpu.VMEM((2, SEG, D), BF16),
            pltpu.VMEM((RA, RA), F32),
            pltpu.SemaphoreType.DMA((XR,)),
            pltpu.SemaphoreType.DMA,
            pltpu.SemaphoreType.DMA((2 * NCH,)),
            pltpu.SemaphoreType.DMA((3 + NQ,)),
            pltpu.SemaphoreType.DMA((2,)),
        ],
        compiler_params=pltpu.CompilerParams(vmem_limit_bytes=126 * 1024 * 1024, disable_bounds_checks=True, disable_semaphore_checks=True),
    )(x, mem0, A_Wq, A_Wk, A_Wv, wo, B_w_gate, B_w_up, B_w_down)
    return out.reshape(1, S, D)
```

```python
import jax
import jax.numpy as jnp
import jax.experimental.pallas as pl
import jax.experimental.pallas.tpu as pltpu

F32 = jnp.float32
BF16 = jnp.bfloat16
U32 = jnp.uint32

S, D, H, DH, M, SEG, FF = 2048, 1024, 32, 128, 8, 32, 3584
NSEG = S // SEG
KT = D // 128
FT = FF // 128
RA = 2 * M + 2 * SEG
RB = 2 * SEG
NSTEP = NSEG + 3
DCH = 128
NCH = D // DCH
NPRE = 10
PRE0 = 2
XR = 16
XPF = 13
NQ = 4
EPS = 1e-5
NEG_REF = -1e9


def _ln(x):
    m = jnp.mean(x, axis=-1, keepdims=True)
    xc = x - m
    v = jnp.mean(xc * xc, axis=-1, keepdims=True)
    return xc * jax.lax.rsqrt(v + EPS)


def _pack(x):
    return pltpu.bitcast(x, U32)


def _unpack(x):
    return pltpu.bitcast(x, BF16)


def _cat(ref, n):
    return jnp.concatenate([_unpack(ref[k]) for k in range(n)], axis=1)


def _store_tiles(ref, r0, x):
    rows = x.shape[0]
    for k in range(KT):
        ref[k, r0 // 2:(r0 + rows) // 2, :] = _pack(x[:, k * 128:(k + 1) * 128])


def _recip(x):
    r = pl.reciprocal(x, approx=True)
    return r * (2.0 - x * r)


def _dot(a, b):
    return jnp.dot(a, b, preferred_element_type=F32)


def _fill(rows_layer, rows_pos, n):
    r = jax.lax.broadcasted_iota(jnp.int32, (n, n), 0)
    c = jax.lax.broadcasted_iota(jnp.int32, (n, n), 1)
    same = rows_layer(r) == rows_layer(c)
    ok = (rows_pos(r) < M) | (rows_pos(r) >= rows_pos(c))
    return jnp.where(same, jnp.where(ok, 0.0, NEG_REF), -jnp.inf).astype(F32)


def _kernel(x_hbm, mem0_hbm, wq_hbm, wk_hbm, wv_hbm, wo_hbm, wg_hbm, wu_hbm, wd_hbm,
            out_hbm,
            xr_s, mem0_s, wq_s, wk_s, wv_s, wo_s, wg_s, wu_s, wd_s,
            st3, sto, stg, stu, std,
            ha_s, hb_s, hp_s, pre_s, acc_s, o_s, act_s, x1a_s, x2_s, x2a_s, xb_s, ost_s, mfill_s,
            sem_x, sem_m, sem_st, sem_w, sem_o):
    scale = DH ** -0.5

    def x_copy(seg):
        return pltpu.make_async_copy(x_hbm.at[pl.ds(pl.multiple_of(seg * SEG, SEG), SEG)],
                                     xr_s.at[seg & (XR - 1)], sem_x.at[seg & (XR - 1)])

    def out_copy(t):
        seg = t - 3
        return pltpu.make_async_copy(ost_s.at[t & 1],
                                     out_hbm.at[pl.ds(pl.multiple_of(seg * SEG, SEG), SEG)], sem_o.at[t & 1])

    def c_wo(q):
        n = H * DH // NQ
        r = pl.ds(pl.multiple_of(q * n, n), n)
        return pltpu.make_async_copy(wo_hbm.at[r], sto.at[r], sem_w.at[3 + q])
    c_wg = pltpu.make_async_copy(wg_hbm, stg, sem_w.at[0])
    c_wu = pltpu.make_async_copy(wu_hbm, stu, sem_w.at[1])
    c_wd = pltpu.make_async_copy(wd_hbm, std, sem_w.at[2])

    def conv_cols(src, dst, nrows, ntile):
        def body(c, carry):
            blk = src[pl.ds(pl.multiple_of(c * DCH, DCH), DCH), :]
            rows = pl.ds(pl.multiple_of(c * (DCH // 2), DCH // 2), DCH // 2)
            for j in range(ntile):
                dst[j, rows, :] = _pack(blk[:, j * 128:(j + 1) * 128])
            return carry
        jax.lax.fori_loop(0, nrows // DCH, body, 0)

    cm = pltpu.make_async_copy(mem0_hbm, mem0_s, sem_m)
    for s in range(PRE0, PRE0 + NPRE):
        x_copy(s).start()

    qkv_src = [wq_hbm, wk_hbm, wv_hbm]
    qkv_dst = [wq_s, wk_s, wv_s]

    def st_copy(w, c):
        slot = (w % 2) * NCH + c
        return pltpu.make_async_copy(qkv_src[w].at[pl.ds(pl.multiple_of(c * DCH, DCH), DCH)], st3.at[slot], sem_st.at[slot])

    SUB = 16
    NSUB = DCH // SUB

    sub_id = jax.lax.broadcasted_iota(jnp.int32, (8, DH), 0)

    def transpose8(v):
        for st in (4, 2, 1):
            keep = (sub_id & st) == 0
            nv = list(v)
            for i in range(8):
                if i & st == 0:
                    a, b = v[i], v[i + st]
                    nv[i] = jnp.where(keep, a, pltpu.roll(b, st, 0))
                    nv[i + st] = jnp.where(keep, pltpu.roll(a, 8 - st, 0), b)
            v = nv
        return v

    def convert_sub(w, c, s):
        x = pltpu.bitcast(st3[(w % 2) * NCH + c, s * SUB:(s + 1) * SUB], U32)
        rows = pl.ds(pl.multiple_of(c * (DCH // 2) + s * (SUB // 2), SUB // 2), SUB // 2)
        for g in range(H // 16):
            r = [x[d, g * 8:(g + 1) * 8, :] for d in range(SUB)]
            even = transpose8([(r[2 * j] & jnp.uint32(0xFFFF)) | (r[2 * j + 1] << 16) for j in range(8)])
            odd = transpose8([(r[2 * j] >> 16) | (r[2 * j + 1] & jnp.uint32(0xFFFF0000)) for j in range(8)])
            for i in range(8):
                qkv_dst[w][2 * (g * 8 + i), rows, :] = even[i]
                qkv_dst[w][2 * (g * 8 + i) + 1, rows, :] = odd[i]

    def convert(w, c):
        for s in range(NSUB):
            convert_sub(w, c, s)

    LOOK = 5
    st_copy(0, 0).start()
    for s in range(PRE0, PRE0 + NPRE):
        x_copy(s).wait()
    for c in range(1, LOOK):
        st_copy(0, c).start()
    late_x = list(range(PRE0)) + list(range(PRE0 + NPRE, XPF))
    cm.start()
    for s in late_x:
        x_copy(s).start()
    for s in range(NPRE):
        _store_tiles(hp_s, s * SEG, _ln(xr_s[PRE0 + s].astype(F32)).astype(BF16))

    def store_pre(w, h, r):
        r = _pack(r.astype(BF16))
        for s in range(NPRE):
            pre_s[s, w, h] = r[s * (SEG // 2):(s + 1) * (SEG // 2)]

    order = [(g // NCH, g % NCH) for g in range(LOOK, 3 * NCH)]
    HPC = H // NCH

    def start_wo():
        for q in range(NQ):
            c_wo(q).start()
    hooks = {(1, 3): start_wo, (1, 7): c_wg.start, (2, 3): c_wu.start, (2, 6): c_wd.start}

    def finish(w, c):
        for j in range(HPC):
            h = c * HPC + j
            r = acc_s[w % 2, h]
            store_pre(w, h, r * scale if w == 0 else r)

    for w in range(3):
        def w_body(c, carry, w=w):
            if w == 0:
                for cc in range(NCH):
                    @pl.when(c == cc)
                    def _(cc=cc):
                        st_copy(*order[2 * cc]).start()
                        st_copy(*order[2 * cc + 1]).start()
            for (hw, hc), fn in hooks.items():
                if hw == w:
                    pl.when(c == hc)(fn)
            st_copy(w, c).wait()
            convert(w, c)
            hpc = _unpack(hp_s[c])
            rows = pl.ds(pl.multiple_of(c * (DCH // 2), DCH // 2), DCH // 2)
            for h in range(H):
                part = _dot(hpc, _unpack(qkv_dst[w][h, rows, :]))
                acc_s[w % 2, h] = jnp.where(c > 0, acc_s[w % 2, h], 0.0) + part
            if w > 0:
                finish(w - 1, c)
            return carry
        jax.lax.fori_loop(0, NCH, w_body, 0)
        if w == 0:
            for wc in order[2 * NCH:]:
                st_copy(*wc).start()

    def v_body(c, carry):
        @pl.when(c % (NCH // NQ) == 0)
        def _():
            c_wo(c // (NCH // NQ)).wait()
        finish(2, c)
        for i in range(H // NCH):
            cc = c * (H // NCH) + i
            blk = sto[pl.ds(pl.multiple_of(cc * DCH, DCH), DCH), :]
            rows = pl.ds(pl.multiple_of(cc * (DCH // 2), DCH // 2), DCH // 2)
            for n in range(KT):
                wo_s[n, rows, :] = _pack(blk[:, n * 128:(n + 1) * 128])
        return carry
    jax.lax.fori_loop(0, NCH, v_body, 0)

    mfill_s[...] = _fill(lambda i: jnp.where(i < 2 * M, i // M, (i - 2 * M) // SEG),
                         lambda i: jnp.where(i < 2 * M, i % M, M + (i - 2 * M) % SEG), RA)
    cm.wait()
    for s in range(PRE0):
        x_copy(s).wait()
    x2a_s[...] = jnp.zeros_like(x2a_s)
    x2_s[...] = jnp.zeros_like(x2_s)
    x1a_s[...] = jnp.zeros_like(x1a_s)
    m0 = mem0_s[...]
    _store_tiles(ha_s, 0, jnp.concatenate([m0, m0], axis=0))
    _store_tiles(ha_s, 2 * M, _ln(xr_s[0].astype(F32)).astype(BF16))
    _store_tiles(ha_s, 2 * M + SEG, jnp.zeros((SEG, D), BF16))

    def attention_phase(ha, fill, filler, pre_idx=None):
        allowed = fill == 0.0
        rows = fill.shape[0]

        def qkv(h):
            q = _dot(ha, _unpack(wq_s[h]))
            kk = _dot(ha, _unpack(wk_s[h]))
            v = _dot(ha, _unpack(wv_s[h]))
            res = [(q * scale).astype(BF16), kk.astype(BF16), v.astype(BF16)]
            if pre_idx is not None:
                res = [jnp.concatenate([r[0:2 * M], _unpack(pre_s[pre_idx, w, h]), r[2 * M:]], axis=0)
                       for w, r in enumerate(res)]
            return res

        def probs(q, kk):
            s = jax.lax.dot_general(q, kk, (((1,), (1,)), ((), ())), preferred_element_type=F32)
            s = jnp.where(allowed, s, fill)
            p = jnp.exp(s - jnp.max(s, axis=-1, keepdims=True))
            return (p * _recip(jnp.sum(p, axis=-1, keepdims=True))).astype(BF16)

        qs, ps = {}, {}
        lag = 2 if ha.shape[0] == RA else 3
        for i in range(H + lag):
            if i < H:
                qs[i] = qkv(i)
            else:
                filler(i - H)
            if 0 <= i - 1 < H:
                ps[i - 1] = probs(qs[i - 1][0], qs[i - 1][1])
            if 0 <= i - lag < H:
                o = _dot(ps.pop(i - lag), qs.pop(i - lag)[2])
                o_s[i - lag, 0:rows // 2, :] = _pack(o.astype(BF16))

    def out_proj(rows):
        o = jnp.concatenate([_unpack(o_s[h, 0:rows // 2, :]) for h in range(H)], axis=1)
        return jnp.concatenate([_dot(o, _unpack(wo_s[n])) for n in range(KT)], axis=1)

    def glu_chunk(hb, j):
        rows = hb.shape[0]
        g = _dot(hb, _unpack(wg_s[j]))
        u = _dot(hb, _unpack(wu_s[j]))
        act_s[j, 0:rows // 2, :] = _pack((jax.nn.sigmoid(g) * u).astype(BF16))

    def glu_down(rows):
        act = jnp.concatenate([_unpack(act_s[j, 0:rows // 2, :]) for j in range(FT)], axis=1)
        return jnp.concatenate([_dot(act, _unpack(wd_s[n])) for n in range(KT)], axis=1)

    def xseg(seg):
        return xr_s[seg & (XR - 1)].astype(F32)

    def full_step(t, use_pre):
        x1a = x1a_s[...]
        x2a = x2a_s[...]
        _store_tiles(hb_s, 0, _ln(x1a).astype(BF16))
        _store_tiles(hb_s, SEG, _ln(x2a).astype(BF16))
        if use_pre:
            ha = jnp.concatenate(
                [jnp.concatenate([_unpack(ha_s[k, 0:M, :]), _unpack(ha_s[k, M + SEG // 2:RA // 2, :])], axis=0)
                 for k in range(KT)], axis=1)
            pre_idx = jnp.clip(t - PRE0, 0, NPRE - 1)
        else:
            ha = _cat(ha_s, KT)
            pre_idx = None
        hb = _cat(hb_s, KT)

        def filler(i):
            glu_chunk(hb, 2 * i)
            glu_chunk(hb, 2 * i + 1)
        attention_phase(ha, mfill_s[...], filler, pre_idx)
        for j in range(6 if use_pre else 4, FT):
            glu_chunk(hb, j)
        z = glu_down(RB)

        xin = xseg(t)
        x2_old = x2_s[...]
        x2_new = x1a + z[0:SEG]
        x2_s[...] = x2_new
        ost_s[t & 1] = (x2a + z[SEG:RB]).astype(BF16)
        n1 = _ln(xseg(jnp.minimum(t + 1, NSEG - 1))).astype(BF16)
        n2 = _ln(x2_new).astype(BF16)

        y = out_proj(RA)
        _store_tiles(ha_s, 0, y[0:2 * M].astype(BF16))
        _store_tiles(ha_s, 2 * M, n1)
        _store_tiles(ha_s, 2 * M + SEG, n2)
        x1a_s[...] = xin + y[2 * M:2 * M + SEG]
        x2a_s[...] = x2_old + y[2 * M + SEG:RA]

    RH = 2 * M + SEG

    def a_half(layer):
        tok0 = M + (SEG // 2) * layer
        ha = jnp.concatenate(
            [jnp.concatenate([_unpack(ha_s[k, 0:M, :]), _unpack(ha_s[k, tok0:tok0 + SEG // 2, :])], axis=0)
             for k in range(KT)], axis=1)
        fill = _fill(lambda i: jnp.where(i < 2 * M, i // M, layer),
                     lambda i: jnp.where(i < 2 * M, i % M, M + i - 2 * M), RH)
        attention_phase(ha, fill, lambda i: None)
        return out_proj(RH)

    def head_step(t):
        xb_s[...] = x1a_s[...]
        y = a_half(0)
        m0f = mem0_s[...].astype(F32)
        _store_tiles(ha_s, 0, jnp.concatenate([y[0:M], m0f], axis=0).astype(BF16))
        _store_tiles(ha_s, 2 * M, _ln(xseg(t + 1)).astype(BF16))
        x1a_s[...] = xseg(t) + y[2 * M:RH]

        @pl.when(t == 1)
        def _():
            c_wg.wait()
            conv_cols(stg, wg_s, D, FT)
            c_wu.wait()
            conv_cols(stu, wu_s, D, FT)
            xb = xb_s[...]
            hb = _ln(xb).astype(BF16)
            for j in range(FT):
                glu_chunk(hb, j)
            c_wd.wait()
            conv_cols(std, wd_s, FF, KT)
            res = xb_s[...] + glu_down(SEG)
            x2_s[...] = res
            _store_tiles(ha_s, 2 * M + SEG, _ln(res).astype(BF16))

    def tail_step(t):
        first = t == NSEG
        xb_s[...] = jnp.where(first, x1a_s[...], x2a_s[...])
        y_old = x2a_s[...]
        y = a_half(1)
        _store_tiles(ha_s, 0, y[0:2 * M].astype(BF16))
        x2a_new = x2_s[...] + y[2 * M:RH]
        x2a_s[...] = x2a_new
        xin0 = xb_s[...]
        xin1 = jnp.where(first, y_old, x2a_new)
        hb = jnp.concatenate([_ln(xin0).astype(BF16), _ln(xin1).astype(BF16)], axis=0)
        for j in range(FT):
            glu_chunk(hb, j)
        z = glu_down(RB)
        res0 = xin0 + z[0:SEG]
        res1 = xin1 + z[SEG:RB]

        @pl.when(first)
        def _():
            x2_s[...] = res0
            _store_tiles(ha_s, 2 * M + SEG, _ln(res0).astype(BF16))
            out_copy(t - 2).wait()
            ost_s[0] = res1.astype(BF16)
            out_copy(t).start()

        @pl.when(jnp.logical_not(first))
        def _():
            out_copy(t - 2).wait()
            ost_s[1] = res0.astype(BF16)
            out_copy(t).start()
            out_copy(t - 1).wait()
            ost_s[0] = res1.astype(BF16)
            out_copy(t + 1).start()

    def x_next(t):
        seg = jnp.minimum(t, NSEG - 1)
        return pltpu.make_async_copy(x_hbm.at[pl.ds(pl.multiple_of(seg * SEG, SEG), SEG)],
                                     xr_s.at[t & (XR - 1)], sem_x.at[t & (XR - 1)])

    def head_body(t, carry):
        x_copy(t + XPF).start()
        head_step(t)
        return carry

    def pre_body_step(t, carry):
        @pl.when(t >= 5)
        def _():
            out_copy(t - 2).wait()

        @pl.when(t + 1 >= PRE0 + NPRE)
        def _():
            x_copy(t + 1).wait()
        x_copy(t + XPF).start()
        full_step(t, True)

        @pl.when(t >= 3)
        def _():
            out_copy(t).start()
        return carry

    def full_body(t, carry):
        out_copy(t - 2).wait()
        x_next(t + 1).wait()
        x_next(t + XPF).start()
        full_step(t, False)
        out_copy(t).start()
        return carry

    def tail_body(t, carry):
        tail_step(t)
        return carry

    jax.lax.fori_loop(0, 2, head_body, 0)
    jax.lax.fori_loop(PRE0, PRE0 + NPRE, pre_body_step, 0)
    jax.lax.fori_loop(PRE0 + NPRE, NSEG, full_body, 0)
    jax.lax.fori_loop(NSEG, NSEG + 2, tail_body, 0)
    for s in range(NSEG + 1, NSEG + XPF):
        x_next(s).wait()
    out_copy(NSTEP - 2).wait()
    out_copy(NSTEP - 1).wait()


@jax.jit
def pallas_interleave_layers__memory_aug_recurrent_mem_tr__glu_gated_glu__prompt_kernel(A_x, A_mem0, A_Wq, A_Wk, A_Wv, A_Wo, A_seg_len, B_x, B_w_gate, B_w_up, B_w_down):
    x = A_x.reshape(S, D)
    mem0 = A_mem0.reshape(M, D)
    wo = A_Wo.reshape(H * DH, D)
    any_spec = pl.BlockSpec(memory_space=pl.ANY)
    out = pl.pallas_call(
        _kernel,
        out_shape=jax.ShapeDtypeStruct((S, D), BF16),
        in_specs=[any_spec] * 9,
        out_specs=any_spec,
        scratch_shapes=[
            pltpu.VMEM((XR, SEG, D), BF16),
            pltpu.VMEM((M, D), BF16),
            pltpu.VMEM((H, D // 2, DH), U32),
            pltpu.VMEM((H, D // 2, DH), U32),
            pltpu.VMEM((H, D // 2, DH), U32),
            pltpu.VMEM((KT, H * DH // 2, 128), U32),
            pltpu.VMEM((FT, D // 2, 128), U32),
            pltpu.VMEM((FT, D // 2, 128), U32),
            pltpu.VMEM((KT, FF // 2, 128), U32),
            pltpu.VMEM((2 * NCH, DCH, H, DH), BF16),
            pltpu.VMEM((H * DH, D), BF16),
            pltpu.VMEM((D, FF), BF16),
            pltpu.VMEM((D, FF), BF16),
            pltpu.VMEM((FF, D), BF16),
            pltpu.VMEM((KT, RA // 2, 128), U32),
            pltpu.VMEM((KT, RB // 2, 128), U32),
            pltpu.VMEM((KT, NPRE * SEG // 2, 128), U32),
            pltpu.VMEM((NPRE, 3, H, SEG // 2, 128), U32),
            pltpu.VMEM((2, H, NPRE * SEG, DH), F32),
            pltpu.VMEM((H, RA // 2, 128), U32),
            pltpu.VMEM((FT, RB // 2, 128), U32),
            pltpu.VMEM((SEG, D), F32),
            pltpu.VMEM((SEG, D), F32),
            pltpu.VMEM((SEG, D), F32),
            pltpu.VMEM((SEG, D), F32),
            pltpu.VMEM((2, SEG, D), BF16),
            pltpu.VMEM((RA, RA), F32),
            pltpu.SemaphoreType.DMA((XR,)),
            pltpu.SemaphoreType.DMA,
            pltpu.SemaphoreType.DMA((2 * NCH,)),
            pltpu.SemaphoreType.DMA((3 + NQ,)),
            pltpu.SemaphoreType.DMA((2,)),
        ],
        compiler_params=pltpu.CompilerParams(vmem_limit_bytes=126 * 1024 * 1024, disable_bounds_checks=True, disable_semaphore_checks=True),
    )(x, mem0, A_Wq, A_Wk, A_Wv, wo, B_w_gate, B_w_up, B_w_down)
    return out.reshape(1, S, D)
```

```python
import jax
import jax.numpy as jnp
import jax.experimental.pallas as pl
import jax.experimental.pallas.tpu as pltpu

F32 = jnp.float32
BF16 = jnp.bfloat16
U32 = jnp.uint32

S, D, H, DH, M, SEG, FF = 2048, 1024, 32, 128, 8, 32, 3584
NSEG = S // SEG
KT = D // 128
FT = FF // 128
RA = 2 * M + 2 * SEG
RB = 2 * SEG
NSTEP = NSEG + 3
DCH = 128
NCH = D // DCH
NPRE = 10
PRE0 = 2
XR = 16
XPF = 13
NQ = 4
EPS = 1e-5
NEG_REF = -1e9


def _ln(x):
    m = jnp.mean(x, axis=-1, keepdims=True)
    xc = x - m
    v = jnp.mean(xc * xc, axis=-1, keepdims=True)
    return xc * jax.lax.rsqrt(v + EPS)


def _pack(x):
    return pltpu.bitcast(x, U32)


def _unpack(x):
    return pltpu.bitcast(x, BF16)


def _cat(ref, n):
    return jnp.concatenate([_unpack(ref[k]) for k in range(n)], axis=1)


def _store_tiles(ref, r0, x):
    rows = x.shape[0]
    for k in range(KT):
        ref[k, r0 // 2:(r0 + rows) // 2, :] = _pack(x[:, k * 128:(k + 1) * 128])


def _recip(x):
    r = pl.reciprocal(x, approx=True)
    return r * (2.0 - x * r)


def _dot(a, b):
    return jnp.dot(a, b, preferred_element_type=F32)


def _fill(rows_layer, rows_pos, n):
    r = jax.lax.broadcasted_iota(jnp.int32, (n, n), 0)
    c = jax.lax.broadcasted_iota(jnp.int32, (n, n), 1)
    same = rows_layer(r) == rows_layer(c)
    ok = (rows_pos(r) < M) | (rows_pos(r) >= rows_pos(c))
    return jnp.where(same, jnp.where(ok, 0.0, NEG_REF), -jnp.inf).astype(F32)


def _kernel(x_hbm, mem0_hbm, wq_hbm, wk_hbm, wv_hbm, wo_hbm, wg_hbm, wu_hbm, wd_hbm,
            out_hbm,
            xr_s, mem0_s, wq_s, wk_s, wv_s, wo_s, wg_s, wu_s, wd_s,
            st3, sto, stg, stu, std,
            ha_s, hb_s, hp_s, pre_s, acc_s, o_s, act_s, x1a_s, x2_s, x2a_s, xb_s, ost_s, mfill_s,
            sem_x, sem_m, sem_st, sem_w, sem_o):
    scale = DH ** -0.5

    def x_copy(seg):
        return pltpu.make_async_copy(x_hbm.at[pl.ds(pl.multiple_of(seg * SEG, SEG), SEG)],
                                     xr_s.at[seg & (XR - 1)], sem_x.at[seg & (XR - 1)])

    def out_copy(t):
        seg = t - 3
        return pltpu.make_async_copy(ost_s.at[t & 1],
                                     out_hbm.at[pl.ds(pl.multiple_of(seg * SEG, SEG), SEG)], sem_o.at[t & 1])

    def c_wo(q):
        n = H * DH // NQ
        r = pl.ds(pl.multiple_of(q * n, n), n)
        return pltpu.make_async_copy(wo_hbm.at[r], sto.at[r], sem_w.at[3 + q])
    c_wg = pltpu.make_async_copy(wg_hbm, stg, sem_w.at[0])
    c_wu = pltpu.make_async_copy(wu_hbm, stu, sem_w.at[1])
    c_wd = pltpu.make_async_copy(wd_hbm, std, sem_w.at[2])

    def conv_cols(src, dst, nrows, ntile):
        def body(c, carry):
            blk = src[pl.ds(pl.multiple_of(c * DCH, DCH), DCH), :]
            rows = pl.ds(pl.multiple_of(c * (DCH // 2), DCH // 2), DCH // 2)
            for j in range(ntile):
                dst[j, rows, :] = _pack(blk[:, j * 128:(j + 1) * 128])
            return carry
        jax.lax.fori_loop(0, nrows // DCH, body, 0)

    cm = pltpu.make_async_copy(mem0_hbm, mem0_s, sem_m)
    for s in range(PRE0, PRE0 + NPRE):
        x_copy(s).start()

    qkv_src = [wq_hbm, wk_hbm, wv_hbm]
    qkv_dst = [wq_s, wk_s, wv_s]

    def st_copy(w, c):
        slot = (w % 2) * NCH + c
        return pltpu.make_async_copy(qkv_src[w].at[pl.ds(pl.multiple_of(c * DCH, DCH), DCH)], st3.at[slot], sem_st.at[slot])

    SUB = 16
    NSUB = DCH // SUB

    sub_id = jax.lax.broadcasted_iota(jnp.int32, (8, DH), 0)

    def transpose8(v):
        for st in (4, 2, 1):
            keep = (sub_id & st) == 0
            nv = list(v)
            for i in range(8):
                if i & st == 0:
                    a, b = v[i], v[i + st]
                    nv[i] = jnp.where(keep, a, pltpu.roll(b, st, 0))
                    nv[i + st] = jnp.where(keep, pltpu.roll(a, 8 - st, 0), b)
            v = nv
        return v

    def convert_sub(w, c, s):
        x = pltpu.bitcast(st3[(w % 2) * NCH + c, s * SUB:(s + 1) * SUB], U32)
        rows = pl.ds(pl.multiple_of(c * (DCH // 2) + s * (SUB // 2), SUB // 2), SUB // 2)
        for g in range(H // 16):
            r = [x[d, g * 8:(g + 1) * 8, :] for d in range(SUB)]
            even = transpose8([(r[2 * j] & jnp.uint32(0xFFFF)) | (r[2 * j + 1] << 16) for j in range(8)])
            odd = transpose8([(r[2 * j] >> 16) | (r[2 * j + 1] & jnp.uint32(0xFFFF0000)) for j in range(8)])
            for i in range(8):
                qkv_dst[w][2 * (g * 8 + i), rows, :] = even[i]
                qkv_dst[w][2 * (g * 8 + i) + 1, rows, :] = odd[i]

    def convert(w, c):
        for s in range(NSUB):
            convert_sub(w, c, s)

    LOOK = 5
    st_copy(0, 0).start()
    for s in range(PRE0, PRE0 + NPRE):
        x_copy(s).wait()
    for c in range(1, LOOK):
        st_copy(0, c).start()
    late_x = list(range(PRE0)) + list(range(PRE0 + NPRE, XPF))
    cm.start()
    for s in late_x:
        x_copy(s).start()
    for s in range(NPRE):
        _store_tiles(hp_s, s * SEG, _ln(xr_s[PRE0 + s].astype(F32)).astype(BF16))

    def store_pre(w, h, r):
        r = _pack(r.astype(BF16))
        for s in range(NPRE):
            pre_s[s, w, h] = r[s * (SEG // 2):(s + 1) * (SEG // 2)]

    order = [(g // NCH, g % NCH) for g in range(LOOK, 3 * NCH)]
    HPC = H // NCH

    def start_wo():
        for q in range(NQ):
            c_wo(q).start()
    hooks = {(1, 3): start_wo, (1, 7): c_wg.start, (2, 3): c_wu.start, (2, 6): c_wd.start}

    def finish(w, c):
        for j in range(HPC):
            h = c * HPC + j
            r = acc_s[w % 2, h]
            store_pre(w, h, r * scale if w == 0 else r)

    for w in range(3):
        def w_body(c, carry, w=w):
            if w == 0:
                for cc in range(NCH):
                    @pl.when(c == cc)
                    def _(cc=cc):
                        st_copy(*order[2 * cc]).start()
                        st_copy(*order[2 * cc + 1]).start()
            for (hw, hc), fn in hooks.items():
                if hw == w:
                    pl.when(c == hc)(fn)
            st_copy(w, c).wait()
            convert(w, c)
            hpc = _unpack(hp_s[c])
            rows = pl.ds(pl.multiple_of(c * (DCH // 2), DCH // 2), DCH // 2)
            for h in range(H):
                part = _dot(hpc, _unpack(qkv_dst[w][h, rows, :]))
                acc_s[w % 2, h] = jnp.where(c > 0, acc_s[w % 2, h], 0.0) + part
            if w > 0:
                finish(w - 1, c)
            return carry
        jax.lax.fori_loop(0, NCH, w_body, 0)
        if w == 0:
            for wc in order[2 * NCH:]:
                st_copy(*wc).start()

    def v_body(c, carry):
        @pl.when(c % (NCH // NQ) == 0)
        def _():
            c_wo(c // (NCH // NQ)).wait()
        finish(2, c)
        for i in range(H // NCH):
            cc = c * (H // NCH) + i
            blk = sto[pl.ds(pl.multiple_of(cc * DCH, DCH), DCH), :]
            rows = pl.ds(pl.multiple_of(cc * (DCH // 2), DCH // 2), DCH // 2)
            for n in range(KT):
                wo_s[n, rows, :] = _pack(blk[:, n * 128:(n + 1) * 128])
        return carry
    jax.lax.fori_loop(0, NCH, v_body, 0)

    mfill_s[...] = _fill(lambda i: jnp.where(i < 2 * M, i // M, (i - 2 * M) // SEG),
                         lambda i: jnp.where(i < 2 * M, i % M, M + (i - 2 * M) % SEG), RA)
    cm.wait()
    for s in range(PRE0):
        x_copy(s).wait()
    x2a_s[...] = jnp.zeros_like(x2a_s)
    x2_s[...] = jnp.zeros_like(x2_s)
    x1a_s[...] = jnp.zeros_like(x1a_s)
    m0 = mem0_s[...]
    _store_tiles(ha_s, 0, jnp.concatenate([m0, m0], axis=0))
    _store_tiles(ha_s, 2 * M, _ln(xr_s[0].astype(F32)).astype(BF16))
    _store_tiles(ha_s, 2 * M + SEG, jnp.zeros((SEG, D), BF16))

    def attention_phase(ha, fill, filler, pre_idx=None):
        allowed = fill == 0.0
        rows = fill.shape[0]

        def qkv(h):
            q = _dot(ha, _unpack(wq_s[h]))
            kk = _dot(ha, _unpack(wk_s[h]))
            v = _dot(ha, _unpack(wv_s[h]))
            res = [(q * scale).astype(BF16), kk.astype(BF16), v.astype(BF16)]
            if pre_idx is not None:
                res = [jnp.concatenate([r[0:2 * M], _unpack(pre_s[pre_idx, w, h]), r[2 * M:]], axis=0)
                       for w, r in enumerate(res)]
            return res

        def probs(q, kk):
            s = jax.lax.dot_general(q, kk, (((1,), (1,)), ((), ())), preferred_element_type=F32)
            s = jnp.where(allowed, s, fill)
            p = jnp.exp(s - jnp.max(s, axis=-1, keepdims=True))
            return (p * _recip(jnp.sum(p, axis=-1, keepdims=True))).astype(BF16)

        qs, ps = {}, {}
        lag = 2 if ha.shape[0] == RA else 3
        for i in range(H + lag):
            if i < H:
                qs[i] = qkv(i)
            else:
                filler(i - H)
            if 0 <= i - 1 < H:
                ps[i - 1] = probs(qs[i - 1][0], qs[i - 1][1])
            if 0 <= i - lag < H:
                o = _dot(ps.pop(i - lag), qs.pop(i - lag)[2])
                o_s[i - lag, 0:rows // 2, :] = _pack(o.astype(BF16))

    def out_proj(rows):
        o = jnp.concatenate([_unpack(o_s[h, 0:rows // 2, :]) for h in range(H)], axis=1)
        return jnp.concatenate([_dot(o, _unpack(wo_s[n])) for n in range(KT)], axis=1)

    def glu_chunk(hb, j):
        rows = hb.shape[0]
        g = _dot(hb, _unpack(wg_s[j]))
        u = _dot(hb, _unpack(wu_s[j]))
        act_s[j, 0:rows // 2, :] = _pack((jax.nn.sigmoid(g) * u).astype(BF16))

    def glu_down(rows):
        act = jnp.concatenate([_unpack(act_s[j, 0:rows // 2, :]) for j in range(FT)], axis=1)
        return jnp.concatenate([_dot(act, _unpack(wd_s[n])) for n in range(KT)], axis=1)

    def xseg(seg):
        return xr_s[seg & (XR - 1)].astype(F32)

    def full_step(t, use_pre, with_glu=True):
        if with_glu:
            x1a = x1a_s[...]
            x2a = x2a_s[...]
            _store_tiles(hb_s, 0, _ln(x1a).astype(BF16))
            _store_tiles(hb_s, SEG, _ln(x2a).astype(BF16))
            hb = _cat(hb_s, KT)
        if use_pre:
            ha = jnp.concatenate(
                [jnp.concatenate([_unpack(ha_s[k, 0:M, :]), _unpack(ha_s[k, M + SEG // 2:RA // 2, :])], axis=0)
                 for k in range(KT)], axis=1)
            pre_idx = jnp.clip(t - PRE0, 0, NPRE - 1)
        else:
            ha = _cat(ha_s, KT)
            pre_idx = None

        done = []

        def filler(i):
            if with_glu:
                glu_chunk(hb, 2 * i)
                glu_chunk(hb, 2 * i + 1)
                done.extend([2 * i, 2 * i + 1])
        attention_phase(ha, mfill_s[...], filler, pre_idx)
        x2_old = x2_s[...]
        if with_glu:
            for j in range(len(done), FT):
                glu_chunk(hb, j)
            z = glu_down(RB)
            x2_new = x1a + z[0:SEG]
            ost_s[t & 1] = (x2a + z[SEG:RB]).astype(BF16)
        else:
            x2_new = xb_s[...]
        x2_s[...] = x2_new
        xin = xseg(t)
        n1 = _ln(xseg(jnp.minimum(t + 1, NSEG - 1))).astype(BF16)
        n2 = _ln(x2_new).astype(BF16)

        y = out_proj(RA)
        _store_tiles(ha_s, 0, y[0:2 * M].astype(BF16))
        _store_tiles(ha_s, 2 * M, n1)
        _store_tiles(ha_s, 2 * M + SEG, n2)
        x1a_s[...] = xin + y[2 * M:2 * M + SEG]
        x2a_s[...] = x2_old + y[2 * M + SEG:RA]

    RH = 2 * M + SEG

    def a_half(layer):
        tok0 = M + (SEG // 2) * layer
        ha = jnp.concatenate(
            [jnp.concatenate([_unpack(ha_s[k, 0:M, :]), _unpack(ha_s[k, tok0:tok0 + SEG // 2, :])], axis=0)
             for k in range(KT)], axis=1)
        fill = _fill(lambda i: jnp.where(i < 2 * M, i // M, layer),
                     lambda i: jnp.where(i < 2 * M, i % M, M + i - 2 * M), RH)
        attention_phase(ha, fill, lambda i: None)
        return out_proj(RH)

    def head_step(t):
        xb_s[...] = x1a_s[...]
        y = a_half(0)
        m0f = mem0_s[...].astype(F32)
        _store_tiles(ha_s, 0, jnp.concatenate([y[0:M], m0f], axis=0).astype(BF16))
        _store_tiles(ha_s, 2 * M, _ln(xseg(t + 1)).astype(BF16))
        x1a_s[...] = xseg(t) + y[2 * M:RH]

        @pl.when(t == 1)
        def _():
            c_wg.wait()
            conv_cols(stg, wg_s, D, FT)
            c_wu.wait()
            conv_cols(stu, wu_s, D, FT)
            hb = jnp.concatenate([_ln(xb_s[...]).astype(BF16), _ln(x1a_s[...]).astype(BF16)], axis=0)
            for j in range(FT):
                glu_chunk(hb, j)
            c_wd.wait()
            conv_cols(std, wd_s, FF, KT)
            z = glu_down(RB)
            res = xb_s[...] + z[0:SEG]
            x2_s[...] = res
            _store_tiles(ha_s, 2 * M + SEG, _ln(res).astype(BF16))
            xb_s[...] = x1a_s[...] + z[SEG:RB]

    def tail_step(t):
        first = t == NSEG
        xb_s[...] = jnp.where(first, x1a_s[...], x2a_s[...])
        y_old = x2a_s[...]
        y = a_half(1)
        _store_tiles(ha_s, 0, y[0:2 * M].astype(BF16))
        x2a_new = x2_s[...] + y[2 * M:RH]
        x2a_s[...] = x2a_new
        xin0 = xb_s[...]
        xin1 = jnp.where(first, y_old, x2a_new)
        hb = jnp.concatenate([_ln(xin0).astype(BF16), _ln(xin1).astype(BF16)], axis=0)
        for j in range(FT):
            glu_chunk(hb, j)
        z = glu_down(RB)
        res0 = xin0 + z[0:SEG]
        res1 = xin1 + z[SEG:RB]

        @pl.when(first)
        def _():
            x2_s[...] = res0
            _store_tiles(ha_s, 2 * M + SEG, _ln(res0).astype(BF16))
            out_copy(t - 2).wait()
            ost_s[0] = res1.astype(BF16)
            out_copy(t).start()

        @pl.when(jnp.logical_not(first))
        def _():
            out_copy(t - 2).wait()
            ost_s[1] = res0.astype(BF16)
            out_copy(t).start()
            out_copy(t - 1).wait()
            ost_s[0] = res1.astype(BF16)
            out_copy(t + 1).start()

    def x_next(t):
        seg = jnp.minimum(t, NSEG - 1)
        return pltpu.make_async_copy(x_hbm.at[pl.ds(pl.multiple_of(seg * SEG, SEG), SEG)],
                                     xr_s.at[t & (XR - 1)], sem_x.at[t & (XR - 1)])

    def head_body(t, carry):
        x_copy(t + XPF).start()
        head_step(t)
        return carry

    def pre_body_step(t, carry):
        @pl.when(t >= 5)
        def _():
            out_copy(t - 2).wait()

        @pl.when(t + 1 >= PRE0 + NPRE)
        def _():
            x_copy(t + 1).wait()
        x_copy(t + XPF).start()
        full_step(t, True)
        out_copy(t).start()
        return carry

    def full_body(t, carry):
        out_copy(t - 2).wait()
        x_next(t + 1).wait()
        x_next(t + XPF).start()
        full_step(t, False)
        out_copy(t).start()
        return carry

    def tail_body(t, carry):
        tail_step(t)
        return carry

    jax.lax.fori_loop(0, 2, head_body, 0)
    x_copy(PRE0 + XPF).start()
    full_step(PRE0, True, with_glu=False)
    jax.lax.fori_loop(PRE0 + 1, PRE0 + NPRE, pre_body_step, 0)
    jax.lax.fori_loop(PRE0 + NPRE, NSEG, full_body, 0)
    jax.lax.fori_loop(NSEG, NSEG + 2, tail_body, 0)
    for s in range(NSEG + 1, NSEG + XPF):
        x_next(s).wait()
    out_copy(NSTEP - 2).wait()
    out_copy(NSTEP - 1).wait()


@jax.jit
def pallas_interleave_layers__memory_aug_recurrent_mem_tr__glu_gated_glu__prompt_kernel(A_x, A_mem0, A_Wq, A_Wk, A_Wv, A_Wo, A_seg_len, B_x, B_w_gate, B_w_up, B_w_down):
    x = A_x.reshape(S, D)
    mem0 = A_mem0.reshape(M, D)
    wo = A_Wo.reshape(H * DH, D)
    any_spec = pl.BlockSpec(memory_space=pl.ANY)
    out = pl.pallas_call(
        _kernel,
        out_shape=jax.ShapeDtypeStruct((S, D), BF16),
        in_specs=[any_spec] * 9,
        out_specs=any_spec,
        scratch_shapes=[
            pltpu.VMEM((XR, SEG, D), BF16),
            pltpu.VMEM((M, D), BF16),
            pltpu.VMEM((H, D // 2, DH), U32),
            pltpu.VMEM((H, D // 2, DH), U32),
            pltpu.VMEM((H, D // 2, DH), U32),
            pltpu.VMEM((KT, H * DH // 2, 128), U32),
            pltpu.VMEM((FT, D // 2, 128), U32),
            pltpu.VMEM((FT, D // 2, 128), U32),
            pltpu.VMEM((KT, FF // 2, 128), U32),
            pltpu.VMEM((2 * NCH, DCH, H, DH), BF16),
            pltpu.VMEM((H * DH, D), BF16),
            pltpu.VMEM((D, FF), BF16),
            pltpu.VMEM((D, FF), BF16),
            pltpu.VMEM((FF, D), BF16),
            pltpu.VMEM((KT, RA // 2, 128), U32),
            pltpu.VMEM((KT, RB // 2, 128), U32),
            pltpu.VMEM((KT, NPRE * SEG // 2, 128), U32),
            pltpu.VMEM((NPRE, 3, H, SEG // 2, 128), U32),
            pltpu.VMEM((2, H, NPRE * SEG, DH), F32),
            pltpu.VMEM((H, RA // 2, 128), U32),
            pltpu.VMEM((FT, RB // 2, 128), U32),
            pltpu.VMEM((SEG, D), F32),
            pltpu.VMEM((SEG, D), F32),
            pltpu.VMEM((SEG, D), F32),
            pltpu.VMEM((SEG, D), F32),
            pltpu.VMEM((2, SEG, D), BF16),
            pltpu.VMEM((RA, RA), F32),
            pltpu.SemaphoreType.DMA((XR,)),
            pltpu.SemaphoreType.DMA,
            pltpu.SemaphoreType.DMA((2 * NCH,)),
            pltpu.SemaphoreType.DMA((3 + NQ,)),
            pltpu.SemaphoreType.DMA((2,)),
        ],
        compiler_params=pltpu.CompilerParams(vmem_limit_bytes=126 * 1024 * 1024, disable_bounds_checks=True, disable_semaphore_checks=True),
    )(x, mem0, A_Wq, A_Wk, A_Wv, wo, B_w_gate, B_w_up, B_w_down)
    return out.reshape(1, S, D)
```

```python
import jax
import jax.numpy as jnp
import jax.experimental.pallas as pl
import jax.experimental.pallas.tpu as pltpu

F32 = jnp.float32
BF16 = jnp.bfloat16
U32 = jnp.uint32

S, D, H, DH, M, SEG, FF = 2048, 1024, 32, 128, 8, 32, 3584
NSEG = S // SEG
KT = D // 128
FT = FF // 128
RA = 2 * M + 2 * SEG
RB = 2 * SEG
NSTEP = NSEG + 3
DCH = 128
NCH = D // DCH
NPRE = 11
PRE0 = 2
XR = 16
XPF = 14
NQ = 4
EPS = 1e-5
NEG_REF = -1e9


def _ln(x):
    m = jnp.mean(x, axis=-1, keepdims=True)
    xc = x - m
    v = jnp.mean(xc * xc, axis=-1, keepdims=True)
    return xc * jax.lax.rsqrt(v + EPS)


def _pack(x):
    return pltpu.bitcast(x, U32)


def _unpack(x):
    return pltpu.bitcast(x, BF16)


def _cat(ref, n):
    return jnp.concatenate([_unpack(ref[k]) for k in range(n)], axis=1)


def _store_tiles(ref, r0, x):
    rows = x.shape[0]
    for k in range(KT):
        ref[k, r0 // 2:(r0 + rows) // 2, :] = _pack(x[:, k * 128:(k + 1) * 128])


def _recip(x):
    r = pl.reciprocal(x, approx=True)
    return r * (2.0 - x * r)


def _dot(a, b):
    return jnp.dot(a, b, preferred_element_type=F32)


def _fill(rows_layer, rows_pos, n):
    r = jax.lax.broadcasted_iota(jnp.int32, (n, n), 0)
    c = jax.lax.broadcasted_iota(jnp.int32, (n, n), 1)
    same = rows_layer(r) == rows_layer(c)
    ok = (rows_pos(r) < M) | (rows_pos(r) >= rows_pos(c))
    return jnp.where(same, jnp.where(ok, 0.0, NEG_REF), -jnp.inf).astype(F32)


def _kernel(x_hbm, mem0_hbm, wq_hbm, wk_hbm, wv_hbm, wo_hbm, wg_hbm, wu_hbm, wd_hbm,
            out_hbm,
            xr_s, mem0_s, wq_s, wk_s, wv_s, wo_s, wg_s, wu_s, wd_s,
            st3, sto, stg, stu, std,
            ha_s, hb_s, hp_s, pre_s, o_s, act_s, x1a_s, x2_s, x2a_s, xb_s, ost_s, mfill_s,
            sem_x, sem_m, sem_st, sem_w, sem_o):
    scale = DH ** -0.5

    def x_copy(seg):
        return pltpu.make_async_copy(x_hbm.at[pl.ds(pl.multiple_of(seg * SEG, SEG), SEG)],
                                     xr_s.at[seg & (XR - 1)], sem_x.at[seg & (XR - 1)])

    def out_copy(t):
        seg = t - 3
        return pltpu.make_async_copy(ost_s.at[t & 1],
                                     out_hbm.at[pl.ds(pl.multiple_of(seg * SEG, SEG), SEG)], sem_o.at[t & 1])

    def c_wo(q):
        n = H * DH // NQ
        r = pl.ds(pl.multiple_of(q * n, n), n)
        return pltpu.make_async_copy(wo_hbm.at[r], sto.at[r], sem_w.at[3 + q])
    c_wg = pltpu.make_async_copy(wg_hbm, stg, sem_w.at[0])
    c_wu = pltpu.make_async_copy(wu_hbm, stu, sem_w.at[1])
    c_wd = pltpu.make_async_copy(wd_hbm, std, sem_w.at[2])

    cm = pltpu.make_async_copy(mem0_hbm, mem0_s, sem_m)
    for s in range(PRE0, PRE0 + NPRE):
        x_copy(s).start()

    qkv_src = [wq_hbm, wk_hbm, wv_hbm]
    qkv_dst = [wq_s, wk_s, wv_s]

    def st_copy(w, c):
        slot = (w % 2) * NCH + c
        return pltpu.make_async_copy(qkv_src[w].at[pl.ds(pl.multiple_of(c * DCH, DCH), DCH)], st3.at[slot], sem_st.at[slot])

    SUB = 16
    NSUB = DCH // SUB

    sub_id = jax.lax.broadcasted_iota(jnp.int32, (8, DH), 0)

    def transpose8(v):
        for st in (4, 2, 1):
            keep = (sub_id & st) == 0
            nv = list(v)
            for i in range(8):
                if i & st == 0:
                    a, b = v[i], v[i + st]
                    nv[i] = jnp.where(keep, a, pltpu.roll(b, st, 0))
                    nv[i + st] = jnp.where(keep, pltpu.roll(a, 8 - st, 0), b)
            v = nv
        return v

    def convert(w, c):
        for g in range(H // 16):
            for par in range(2):
                for s in range(NSUB):
                    x = pltpu.bitcast(st3[(w % 2) * NCH + c, s * SUB:(s + 1) * SUB], U32)
                    r = [x[d, g * 8:(g + 1) * 8, :] for d in range(SUB)]
                    if par == 0:
                        v = [(r[2 * j] & jnp.uint32(0xFFFF)) | (r[2 * j + 1] << 16) for j in range(8)]
                    else:
                        v = [(r[2 * j] >> 16) | (r[2 * j + 1] & jnp.uint32(0xFFFF0000)) for j in range(8)]
                    v = transpose8(v)
                    rows = pl.ds(pl.multiple_of(c * (DCH // 2) + s * (SUB // 2), SUB // 2), SUB // 2)
                    for i in range(8):
                        qkv_dst[w][2 * (g * 8 + i) + par, rows, :] = v[i]

    LOOK = 5
    st_copy(0, 0).start()
    for s in range(PRE0, PRE0 + NPRE):
        x_copy(s).wait()
    for c in range(1, LOOK):
        st_copy(0, c).start()
    late_x = list(range(PRE0)) + list(range(PRE0 + NPRE, XPF))
    cm.start()
    for s in late_x:
        x_copy(s).start()
    for s in range(NPRE):
        _store_tiles(hp_s, s * SEG, _ln(xr_s[PRE0 + s].astype(F32)).astype(BF16))

    order = [(g // NCH, g % NCH) for g in range(LOOK, 3 * NCH)]

    def start_wo():
        for q in range(NQ):
            c_wo(q).start()
    hooks = {(1, 3): start_wo, (1, 7): c_wg.start, (2, 3): c_wu.start, (2, 6): c_wd.start}

    for w in range(3):
        def w_body(c, carry, w=w):
            if w == 0:
                for cc in range(NCH):
                    @pl.when(c == cc)
                    def _(cc=cc):
                        st_copy(*order[2 * cc]).start()
                        st_copy(*order[2 * cc + 1]).start()
            for (hw, hc), fn in hooks.items():
                if hw == w:
                    pl.when(c == hc)(fn)
            st_copy(w, c).wait()
            convert(w, c)
            hpc = _unpack(hp_s[c])
            rows = pl.ds(pl.multiple_of(c * (DCH // 2), DCH // 2), DCH // 2)
            for h in [g * 16 + 2 * i + par for g in range(H // 16) for par in range(2) for i in range(8)]:
                part = _dot(hpc, _unpack(qkv_dst[w][h, rows, :]))
                pre_s[w, h] = jnp.where(c > 0, pre_s[w, h], 0.0) + part
            return carry
        jax.lax.fori_loop(0, NCH, w_body, 0)
        if w == 0:
            for wc in order[2 * NCH:]:
                st_copy(*wc).start()

    mfill_s[...] = _fill(lambda i: jnp.where(i < 2 * M, i // M, (i - 2 * M) // SEG),
                         lambda i: jnp.where(i < 2 * M, i % M, M + (i - 2 * M) % SEG), RA)
    cm.wait()
    for s in range(PRE0):
        x_copy(s).wait()
    x2a_s[...] = jnp.zeros_like(x2a_s)
    x2_s[...] = jnp.zeros_like(x2_s)
    x1a_s[...] = jnp.zeros_like(x1a_s)
    m0 = mem0_s[...]
    _store_tiles(ha_s, 0, jnp.concatenate([m0, m0], axis=0))
    _store_tiles(ha_s, 2 * M, _ln(xr_s[0].astype(F32)).astype(BF16))
    _store_tiles(ha_s, 2 * M + SEG, jnp.zeros((SEG, D), BF16))

    def attention_phase(ha, fill, filler, pre_idx=None):
        allowed = fill == 0.0
        rows = fill.shape[0]

        def qkv(h):
            q = _dot(ha, _unpack(wq_s[h]))
            kk = _dot(ha, _unpack(wk_s[h]))
            v = _dot(ha, _unpack(wv_s[h]))
            res = [(q * scale).astype(BF16), kk.astype(BF16), v.astype(BF16)]
            if pre_idx is not None:
                rows_p = pl.ds(pl.multiple_of(pre_idx * SEG, SEG), SEG)
                tok = [pre_s[w, h, rows_p, :] for w in range(3)]
                tok = [(tok[0] * scale).astype(BF16), tok[1].astype(BF16), tok[2].astype(BF16)]
                res = [jnp.concatenate([r[0:2 * M], p, r[2 * M:]], axis=0) for p, r in zip(tok, res)]
            return res

        def probs(q, kk):
            s = jax.lax.dot_general(q, kk, (((1,), (1,)), ((), ())), preferred_element_type=F32)
            s = jnp.where(allowed, s, fill)
            p = jnp.exp(s - jnp.max(s, axis=-1, keepdims=True))
            return (p * _recip(jnp.sum(p, axis=-1, keepdims=True))).astype(BF16)

        qs, ps = {}, {}
        lag = 2 if ha.shape[0] == RA else 3
        for i in range(H + lag):
            if i < H:
                qs[i] = qkv(i)
            else:
                filler(i - H)
            if 0 <= i - 1 < H:
                ps[i - 1] = probs(qs[i - 1][0], qs[i - 1][1])
            if 0 <= i - lag < H:
                o = _dot(ps.pop(i - lag), qs.pop(i - lag)[2])
                o_s[i - lag, 0:rows // 2, :] = _pack(o.astype(BF16))

    def tile(dst, j, src):
        if src is None:
            return _unpack(dst[j])
        w = src[:, j * 128:(j + 1) * 128]
        dst[j] = _pack(w)
        return w

    def out_proj(rows, fresh=False):
        o = jnp.concatenate([_unpack(o_s[h, 0:rows // 2, :]) for h in range(H)], axis=1)
        return jnp.concatenate([_dot(o, tile(wo_s, n, sto if fresh else None)) for n in range(KT)], axis=1)

    def glu_chunk(hb, j, fresh=False):
        rows = hb.shape[0]
        g = _dot(hb, tile(wg_s, j, stg if fresh else None))
        u = _dot(hb, tile(wu_s, j, stu if fresh else None))
        act_s[j, 0:rows // 2, :] = _pack((jax.nn.sigmoid(g) * u).astype(BF16))

    def glu_down(rows, fresh=False):
        act = jnp.concatenate([_unpack(act_s[j, 0:rows // 2, :]) for j in range(FT)], axis=1)
        return jnp.concatenate([_dot(act, tile(wd_s, n, std if fresh else None)) for n in range(KT)], axis=1)

    def xseg(seg):
        return xr_s[seg & (XR - 1)].astype(F32)

    def full_step(t, use_pre, with_glu=True):
        if with_glu:
            x1a = x1a_s[...]
            x2a = x2a_s[...]
            _store_tiles(hb_s, 0, _ln(x1a).astype(BF16))
            _store_tiles(hb_s, SEG, _ln(x2a).astype(BF16))
            hb = _cat(hb_s, KT)
        if use_pre:
            ha = jnp.concatenate(
                [jnp.concatenate([_unpack(ha_s[k, 0:M, :]), _unpack(ha_s[k, M + SEG // 2:RA // 2, :])], axis=0)
                 for k in range(KT)], axis=1)
            pre_idx = jnp.clip(t - PRE0, 0, NPRE - 1)
        else:
            ha = _cat(ha_s, KT)
            pre_idx = None

        done = []

        def filler(i):
            if with_glu:
                glu_chunk(hb, 2 * i)
                glu_chunk(hb, 2 * i + 1)
                done.extend([2 * i, 2 * i + 1])
        attention_phase(ha, mfill_s[...], filler, pre_idx)
        x2_old = x2_s[...]
        if with_glu:
            for j in range(len(done), FT):
                glu_chunk(hb, j)
            z = glu_down(RB)
            x2_new = x1a + z[0:SEG]
            ost_s[t & 1] = (x2a + z[SEG:RB]).astype(BF16)
        else:
            x2_new = xb_s[...]
        x2_s[...] = x2_new
        xin = xseg(t)
        n1 = _ln(xseg(jnp.minimum(t + 1, NSEG - 1))).astype(BF16)
        n2 = _ln(x2_new).astype(BF16)

        y = out_proj(RA)
        _store_tiles(ha_s, 0, y[0:2 * M].astype(BF16))
        _store_tiles(ha_s, 2 * M, n1)
        _store_tiles(ha_s, 2 * M + SEG, n2)
        x1a_s[...] = xin + y[2 * M:2 * M + SEG]
        x2a_s[...] = x2_old + y[2 * M + SEG:RA]

    RH = 2 * M + SEG

    def a_half(layer):
        tok0 = M + (SEG // 2) * layer
        ha = jnp.concatenate(
            [jnp.concatenate([_unpack(ha_s[k, 0:M, :]), _unpack(ha_s[k, tok0:tok0 + SEG // 2, :])], axis=0)
             for k in range(KT)], axis=1)
        fill = _fill(lambda i: jnp.where(i < 2 * M, i // M, layer),
                     lambda i: jnp.where(i < 2 * M, i % M, M + i - 2 * M), RH)
        attention_phase(ha, fill, lambda i: None)
        return out_proj(RH, fresh=(layer == 0))

    def head_step(t):
        xb_s[...] = x1a_s[...]

        @pl.when(t == 0)
        def _():
            for q in range(NQ):
                c_wo(q).wait()
        y = a_half(0)
        m0f = mem0_s[...].astype(F32)
        _store_tiles(ha_s, 0, jnp.concatenate([y[0:M], m0f], axis=0).astype(BF16))
        _store_tiles(ha_s, 2 * M, _ln(xseg(t + 1)).astype(BF16))
        x1a_s[...] = xseg(t) + y[2 * M:RH]

        @pl.when(t == 1)
        def _():
            c_wg.wait()
            c_wu.wait()
            hb = jnp.concatenate([_ln(xb_s[...]).astype(BF16), _ln(x1a_s[...]).astype(BF16)], axis=0)
            for j in range(FT):
                glu_chunk(hb, j, fresh=True)
            c_wd.wait()
            z = glu_down(RB, fresh=True)
            res = xb_s[...] + z[0:SEG]
            x2_s[...] = res
            _store_tiles(ha_s, 2 * M + SEG, _ln(res).astype(BF16))
            xb_s[...] = x1a_s[...] + z[SEG:RB]

    def tail_step(t):
        first = t == NSEG
        xb_s[...] = jnp.where(first, x1a_s[...], x2a_s[...])
        y_old = x2a_s[...]
        y = a_half(1)
        _store_tiles(ha_s, 0, y[0:2 * M].astype(BF16))
        x2a_new = x2_s[...] + y[2 * M:RH]
        x2a_s[...] = x2a_new
        xin0 = xb_s[...]
        xin1 = jnp.where(first, y_old, x2a_new)
        hb = jnp.concatenate([_ln(xin0).astype(BF16), _ln(xin1).astype(BF16)], axis=0)
        for j in range(FT):
            glu_chunk(hb, j)
        z = glu_down(RB)
        res0 = xin0 + z[0:SEG]
        res1 = xin1 + z[SEG:RB]

        @pl.when(first)
        def _():
            x2_s[...] = res0
            _store_tiles(ha_s, 2 * M + SEG, _ln(res0).astype(BF16))
            out_copy(t - 2).wait()
            ost_s[0] = res1.astype(BF16)
            out_copy(t).start()

        @pl.when(jnp.logical_not(first))
        def _():
            out_copy(t - 2).wait()
            ost_s[1] = res0.astype(BF16)
            out_copy(t).start()
            out_copy(t - 1).wait()
            ost_s[0] = res1.astype(BF16)
            out_copy(t + 1).start()

    def x_next(t):
        seg = jnp.minimum(t, NSEG - 1)
        return pltpu.make_async_copy(x_hbm.at[pl.ds(pl.multiple_of(seg * SEG, SEG), SEG)],
                                     xr_s.at[t & (XR - 1)], sem_x.at[t & (XR - 1)])

    def head_body(t, carry):
        x_copy(t + XPF).start()
        head_step(t)
        return carry

    def pre_body_step(t, carry):
        @pl.when(t >= 5)
        def _():
            out_copy(t - 2).wait()

        @pl.when(t + 1 >= PRE0 + NPRE)
        def _():
            x_copy(t + 1).wait()
        x_copy(t + XPF).start()
        full_step(t, True)
        out_copy(t).start()
        return carry

    def full_body(t, carry):
        out_copy(t - 2).wait()
        x_next(t + 1).wait()
        x_next(t + XPF).start()
        full_step(t, False)
        out_copy(t).start()
        return carry

    def tail_body(t, carry):
        tail_step(t)
        return carry

    jax.lax.fori_loop(0, 2, head_body, 0)
    x_copy(PRE0 + XPF).start()
    full_step(PRE0, True, with_glu=False)
    jax.lax.fori_loop(PRE0 + 1, PRE0 + NPRE, pre_body_step, 0)
    jax.lax.fori_loop(PRE0 + NPRE, NSEG, full_body, 0)
    jax.lax.fori_loop(NSEG, NSEG + 2, tail_body, 0)
    for s in range(NSEG + 1, NSEG + XPF):
        x_next(s).wait()
    out_copy(NSTEP - 2).wait()
    out_copy(NSTEP - 1).wait()


@jax.jit
def pallas_interleave_layers__memory_aug_recurrent_mem_tr__glu_gated_glu__prompt_kernel(A_x, A_mem0, A_Wq, A_Wk, A_Wv, A_Wo, A_seg_len, B_x, B_w_gate, B_w_up, B_w_down):
    x = A_x.reshape(S, D)
    mem0 = A_mem0.reshape(M, D)
    wo = A_Wo.reshape(H * DH, D)
    any_spec = pl.BlockSpec(memory_space=pl.ANY)
    out = pl.pallas_call(
        _kernel,
        out_shape=jax.ShapeDtypeStruct((S, D), BF16),
        in_specs=[any_spec] * 9,
        out_specs=any_spec,
        scratch_shapes=[
            pltpu.VMEM((XR, SEG, D), BF16),
            pltpu.VMEM((M, D), BF16),
            pltpu.VMEM((H, D // 2, DH), U32),
            pltpu.VMEM((H, D // 2, DH), U32),
            pltpu.VMEM((H, D // 2, DH), U32),
            pltpu.VMEM((KT, H * DH // 2, 128), U32),
            pltpu.VMEM((FT, D // 2, 128), U32),
            pltpu.VMEM((FT, D // 2, 128), U32),
            pltpu.VMEM((KT, FF // 2, 128), U32),
            pltpu.VMEM((2 * NCH, DCH, H, DH), BF16),
            pltpu.VMEM((H * DH, D), BF16),
            pltpu.VMEM((D, FF), BF16),
            pltpu.VMEM((D, FF), BF16),
            pltpu.VMEM((FF, D), BF16),
            pltpu.VMEM((KT, RA // 2, 128), U32),
            pltpu.VMEM((KT, RB // 2, 128), U32),
            pltpu.VMEM((KT, NPRE * SEG // 2, 128), U32),
            pltpu.VMEM((3, H, NPRE * SEG, DH), F32),
            pltpu.VMEM((H, RA // 2, 128), U32),
            pltpu.VMEM((FT, RB // 2, 128), U32),
            pltpu.VMEM((SEG, D), F32),
            pltpu.VMEM((SEG, D), F32),
            pltpu.VMEM((SEG, D), F32),
            pltpu.VMEM((SEG, D), F32),
            pltpu.VMEM((2, SEG, D), BF16),
            pltpu.VMEM((RA, RA), F32),
            pltpu.SemaphoreType.DMA((XR,)),
            pltpu.SemaphoreType.DMA,
            pltpu.SemaphoreType.DMA((2 * NCH,)),
            pltpu.SemaphoreType.DMA((3 + NQ,)),
            pltpu.SemaphoreType.DMA((2,)),
        ],
        compiler_params=pltpu.CompilerParams(vmem_limit_bytes=126 * 1024 * 1024, disable_bounds_checks=True, disable_semaphore_checks=True),
    )(x, mem0, A_Wq, A_Wk, A_Wv, wo, B_w_gate, B_w_up, B_w_down)
    return out.reshape(1, S, D)
```

```python
import jax
import jax.numpy as jnp
import jax.experimental.pallas as pl
import jax.experimental.pallas.tpu as pltpu

F32 = jnp.float32
BF16 = jnp.bfloat16
U32 = jnp.uint32

S, D, H, DH, M, SEG, FF = 2048, 1024, 32, 128, 8, 32, 3584
NSEG = S // SEG
KT = D // 128
FT = FF // 128
RA = 2 * M + 2 * SEG
RB = 2 * SEG
NSTEP = NSEG + 3
DCH = 128
NCH = D // DCH
NPRE = 12
PRE0 = 2
XR = 16
XPF = 15
NQ = 4
EPS = 1e-5
NEG_REF = -1e9


def _ln(x):
    m = jnp.mean(x, axis=-1, keepdims=True)
    xc = x - m
    v = jnp.mean(xc * xc, axis=-1, keepdims=True)
    return xc * jax.lax.rsqrt(v + EPS)


def _pack(x):
    return pltpu.bitcast(x, U32)


def _unpack(x):
    return pltpu.bitcast(x, BF16)


def _cat(ref, n):
    return jnp.concatenate([_unpack(ref[k]) for k in range(n)], axis=1)


def _store_tiles(ref, r0, x):
    rows = x.shape[0]
    for k in range(KT):
        ref[k, r0 // 2:(r0 + rows) // 2, :] = _pack(x[:, k * 128:(k + 1) * 128])


def _recip(x):
    r = pl.reciprocal(x, approx=True)
    return r * (2.0 - x * r)


def _dot(a, b):
    return jnp.dot(a, b, preferred_element_type=F32)


def _fill(rows_layer, rows_pos, n):
    r = jax.lax.broadcasted_iota(jnp.int32, (n, n), 0)
    c = jax.lax.broadcasted_iota(jnp.int32, (n, n), 1)
    same = rows_layer(r) == rows_layer(c)
    ok = (rows_pos(r) < M) | (rows_pos(r) >= rows_pos(c))
    return jnp.where(same, jnp.where(ok, 0.0, NEG_REF), -jnp.inf).astype(F32)


def _kernel(x_hbm, mem0_hbm, wq_hbm, wk_hbm, wv_hbm, wo_hbm, wg_hbm, wu_hbm, wd_hbm,
            out_hbm,
            xr_s, mem0_s, wq_s, wk_s, wv_s, wo_s, wg_s, wu_s, wd_s,
            st3, sto, stg, stu, std,
            ha_s, hb_s, hp_s, pre_s, o_s, act_s, x1a_s, x2_s, x2a_s, xb_s, ost_s, mfill_s,
            sem_x, sem_m, sem_st, sem_w, sem_o):
    scale = DH ** -0.5

    def x_copy(seg):
        return pltpu.make_async_copy(x_hbm.at[pl.ds(pl.multiple_of(seg * SEG, SEG), SEG)],
                                     xr_s.at[seg & (XR - 1)], sem_x.at[seg & (XR - 1)])

    def out_copy(t):
        seg = t - 3
        return pltpu.make_async_copy(ost_s.at[t & 1],
                                     out_hbm.at[pl.ds(pl.multiple_of(seg * SEG, SEG), SEG)], sem_o.at[t & 1])

    def c_wo(q):
        n = H * DH // NQ
        r = pl.ds(pl.multiple_of(q * n, n), n)
        return pltpu.make_async_copy(wo_hbm.at[r], sto.at[r], sem_w.at[3 + q])
    c_wg = pltpu.make_async_copy(wg_hbm, stg, sem_w.at[0])
    c_wu = pltpu.make_async_copy(wu_hbm, stu, sem_w.at[1])
    c_wd = pltpu.make_async_copy(wd_hbm, std, sem_w.at[2])

    cm = pltpu.make_async_copy(mem0_hbm, mem0_s, sem_m)
    for s in range(PRE0, PRE0 + NPRE):
        x_copy(s).start()

    qkv_src = [wq_hbm, wk_hbm, wv_hbm]
    qkv_dst = [wq_s, wk_s, wv_s]

    def st_copy(w, c):
        slot = (w % 2) * NCH + c
        return pltpu.make_async_copy(qkv_src[w].at[pl.ds(pl.multiple_of(c * DCH, DCH), DCH)], st3.at[slot], sem_st.at[slot])

    SUB = 16
    NSUB = DCH // SUB

    sub_id = jax.lax.broadcasted_iota(jnp.int32, (8, DH), 0)

    def transpose8(v):
        for st in (4, 2, 1):
            keep = (sub_id & st) == 0
            nv = list(v)
            for i in range(8):
                if i & st == 0:
                    a, b = v[i], v[i + st]
                    nv[i] = jnp.where(keep, a, pltpu.roll(b, st, 0))
                    nv[i + st] = jnp.where(keep, pltpu.roll(a, 8 - st, 0), b)
            v = nv
        return v

    def convert(w, c):
        for g in range(H // 16):
            for par in range(2):
                for s in range(NSUB):
                    x = pltpu.bitcast(st3[(w % 2) * NCH + c, s * SUB:(s + 1) * SUB], U32)
                    r = [x[d, g * 8:(g + 1) * 8, :] for d in range(SUB)]
                    if par == 0:
                        v = [(r[2 * j] & jnp.uint32(0xFFFF)) | (r[2 * j + 1] << 16) for j in range(8)]
                    else:
                        v = [(r[2 * j] >> 16) | (r[2 * j + 1] & jnp.uint32(0xFFFF0000)) for j in range(8)]
                    v = transpose8(v)
                    rows = pl.ds(pl.multiple_of(c * (DCH // 2) + s * (SUB // 2), SUB // 2), SUB // 2)
                    for i in range(8):
                        qkv_dst[w][2 * (g * 8 + i) + par, rows, :] = v[i]

    LOOK = 5
    st_copy(0, 0).start()
    for s in range(PRE0, PRE0 + NPRE):
        x_copy(s).wait()
    for c in range(1, LOOK):
        st_copy(0, c).start()
    late_x = list(range(PRE0)) + list(range(PRE0 + NPRE, XPF))
    cm.start()
    for s in late_x:
        x_copy(s).start()
    for s in range(NPRE):
        _store_tiles(hp_s, s * SEG, _ln(xr_s[PRE0 + s].astype(F32)).astype(BF16))

    order = [(g // NCH, g % NCH) for g in range(LOOK, 3 * NCH)]

    def start_wo():
        for q in range(NQ):
            c_wo(q).start()
    hooks = {(1, 3): start_wo, (1, 7): c_wg.start, (2, 3): c_wu.start, (2, 6): c_wd.start}
    head_order = [g * 16 + 2 * i + par for g in range(H // 16) for par in range(2) for i in range(8)]

    for w in range(3):
        nc = 1 if w == 0 else 2

        def w_body(it, carry, w=w, nc=nc):
            c0 = it * nc
            if w == 0:
                for cc in range(NCH):
                    @pl.when(it == cc)
                    def _(cc=cc):
                        st_copy(*order[2 * cc]).start()
                        st_copy(*order[2 * cc + 1]).start()
            for (hw, hc), fn in hooks.items():
                if hw == w:
                    pl.when(it == hc // nc)(fn)
            for k in range(nc):
                st_copy(w, c0 + k).wait()
            for k in range(nc):
                convert(w, c0 + k)
            hpc = jnp.concatenate([_unpack(hp_s[c0 + k]) for k in range(nc)], axis=1)
            rows = pl.ds(pl.multiple_of(c0 * (DCH // 2), DCH // 2), nc * DCH // 2)
            for h in head_order:
                part = _dot(hpc, _unpack(qkv_dst[w][h, rows, :]))
                pre_s[w, h] = jnp.where(it > 0, pre_s[w, h], 0.0) + part
            return carry
        jax.lax.fori_loop(0, NCH // nc, w_body, 0)
        if w == 0:
            for wc in order[2 * NCH:]:
                st_copy(*wc).start()

    mfill_s[...] = _fill(lambda i: jnp.where(i < 2 * M, i // M, (i - 2 * M) // SEG),
                         lambda i: jnp.where(i < 2 * M, i % M, M + (i - 2 * M) % SEG), RA)
    cm.wait()
    for s in range(PRE0):
        x_copy(s).wait()
    x2a_s[...] = jnp.zeros_like(x2a_s)
    x2_s[...] = jnp.zeros_like(x2_s)
    x1a_s[...] = jnp.zeros_like(x1a_s)
    m0 = mem0_s[...]
    _store_tiles(ha_s, 0, jnp.concatenate([m0, m0], axis=0))
    _store_tiles(ha_s, 2 * M, _ln(xr_s[0].astype(F32)).astype(BF16))
    _store_tiles(ha_s, 2 * M + SEG, jnp.zeros((SEG, D), BF16))

    def attention_phase(ha, fill, filler, pre_idx=None):
        allowed = fill == 0.0
        rows = fill.shape[0]

        def qkv(h):
            q = _dot(ha, _unpack(wq_s[h]))
            kk = _dot(ha, _unpack(wk_s[h]))
            v = _dot(ha, _unpack(wv_s[h]))
            res = [(q * scale).astype(BF16), kk.astype(BF16), v.astype(BF16)]
            if pre_idx is not None:
                rows_p = pl.ds(pl.multiple_of(pre_idx * SEG, SEG), SEG)
                tok = [pre_s[w, h, rows_p, :] for w in range(3)]
                tok = [(tok[0] * scale).astype(BF16), tok[1].astype(BF16), tok[2].astype(BF16)]
                res = [jnp.concatenate([r[0:2 * M], p, r[2 * M:]], axis=0) for p, r in zip(tok, res)]
            return res

        def probs(q, kk):
            s = jax.lax.dot_general(q, kk, (((1,), (1,)), ((), ())), preferred_element_type=F32)
            s = jnp.where(allowed, s, fill)
            p = jnp.exp(s - jnp.max(s, axis=-1, keepdims=True))
            return (p * _recip(jnp.sum(p, axis=-1, keepdims=True))).astype(BF16)

        qs, ps = {}, {}
        lag = 2 if ha.shape[0] == RA else 3
        for i in range(H + lag):
            if i < H:
                qs[i] = qkv(i)
            else:
                filler(i - H)
            if 0 <= i - 1 < H:
                ps[i - 1] = probs(qs[i - 1][0], qs[i - 1][1])
            if 0 <= i - lag < H:
                o = _dot(ps.pop(i - lag), qs.pop(i - lag)[2])
                o_s[i - lag, 0:rows // 2, :] = _pack(o.astype(BF16))

    def tile(dst, j, src):
        if src is None:
            return _unpack(dst[j])
        w = src[:, j * 128:(j + 1) * 128]
        dst[j] = _pack(w)
        return w

    def out_proj(rows, fresh=False):
        o = jnp.concatenate([_unpack(o_s[h, 0:rows // 2, :]) for h in range(H)], axis=1)
        return jnp.concatenate([_dot(o, tile(wo_s, n, sto if fresh else None)) for n in range(KT)], axis=1)

    def glu_chunk(hb, j, fresh=False):
        rows = hb.shape[0]
        g = _dot(hb, tile(wg_s, j, stg if fresh else None))
        u = _dot(hb, tile(wu_s, j, stu if fresh else None))
        act_s[j, 0:rows // 2, :] = _pack((jax.nn.sigmoid(g) * u).astype(BF16))

    def glu_down(rows, fresh=False):
        act = jnp.concatenate([_unpack(act_s[j, 0:rows // 2, :]) for j in range(FT)], axis=1)
        return jnp.concatenate([_dot(act, tile(wd_s, n, std if fresh else None)) for n in range(KT)], axis=1)

    def xseg(seg):
        return xr_s[seg & (XR - 1)].astype(F32)

    def full_step(t, use_pre, with_glu=True):
        if with_glu:
            x1a = x1a_s[...]
            x2a = x2a_s[...]
            _store_tiles(hb_s, 0, _ln(x1a).astype(BF16))
            _store_tiles(hb_s, SEG, _ln(x2a).astype(BF16))
            hb = _cat(hb_s, KT)
        if use_pre:
            ha = jnp.concatenate(
                [jnp.concatenate([_unpack(ha_s[k, 0:M, :]), _unpack(ha_s[k, M + SEG // 2:RA // 2, :])], axis=0)
                 for k in range(KT)], axis=1)
            pre_idx = jnp.clip(t - PRE0, 0, NPRE - 1)
        else:
            ha = _cat(ha_s, KT)
            pre_idx = None

        done = []

        def filler(i):
            if with_glu:
                glu_chunk(hb, 2 * i)
                glu_chunk(hb, 2 * i + 1)
                done.extend([2 * i, 2 * i + 1])
        attention_phase(ha, mfill_s[...], filler, pre_idx)
        x2_old = x2_s[...]
        if with_glu:
            for j in range(len(done), FT):
                glu_chunk(hb, j)
            z = glu_down(RB)
            x2_new = x1a + z[0:SEG]
            ost_s[t & 1] = (x2a + z[SEG:RB]).astype(BF16)
        else:
            x2_new = xb_s[...]
        x2_s[...] = x2_new
        xin = xseg(t)
        n1 = _ln(xseg(jnp.minimum(t + 1, NSEG - 1))).astype(BF16)
        n2 = _ln(x2_new).astype(BF16)

        y = out_proj(RA)
        _store_tiles(ha_s, 0, y[0:2 * M].astype(BF16))
        _store_tiles(ha_s, 2 * M, n1)
        _store_tiles(ha_s, 2 * M + SEG, n2)
        x1a_s[...] = xin + y[2 * M:2 * M + SEG]
        x2a_s[...] = x2_old + y[2 * M + SEG:RA]

    RH = 2 * M + SEG

    def a_half(layer):
        tok0 = M + (SEG // 2) * layer
        ha = jnp.concatenate(
            [jnp.concatenate([_unpack(ha_s[k, 0:M, :]), _unpack(ha_s[k, tok0:tok0 + SEG // 2, :])], axis=0)
             for k in range(KT)], axis=1)
        fill = _fill(lambda i: jnp.where(i < 2 * M, i // M, layer),
                     lambda i: jnp.where(i < 2 * M, i % M, M + i - 2 * M), RH)
        attention_phase(ha, fill, lambda i: None)
        return out_proj(RH, fresh=(layer == 0))

    def head_step(t):
        xb_s[...] = x1a_s[...]

        @pl.when(t == 0)
        def _():
            for q in range(NQ):
                c_wo(q).wait()
        y = a_half(0)
        m0f = mem0_s[...].astype(F32)
        _store_tiles(ha_s, 0, jnp.concatenate([y[0:M], m0f], axis=0).astype(BF16))
        _store_tiles(ha_s, 2 * M, _ln(xseg(t + 1)).astype(BF16))
        x1a_s[...] = xseg(t) + y[2 * M:RH]

        @pl.when(t == 1)
        def _():
            c_wg.wait()
            c_wu.wait()
            hb = jnp.concatenate([_ln(xb_s[...]).astype(BF16), _ln(x1a_s[...]).astype(BF16)], axis=0)
            for j in range(FT):
                glu_chunk(hb, j, fresh=True)
            c_wd.wait()
            z = glu_down(RB, fresh=True)
            res = xb_s[...] + z[0:SEG]
            x2_s[...] = res
            _store_tiles(ha_s, 2 * M + SEG, _ln(res).astype(BF16))
            xb_s[...] = x1a_s[...] + z[SEG:RB]

    def tail_step(t):
        first = t == NSEG
        xb_s[...] = jnp.where(first, x1a_s[...], x2a_s[...])
        y_old = x2a_s[...]
        y = a_half(1)
        _store_tiles(ha_s, 0, y[0:2 * M].astype(BF16))
        x2a_new = x2_s[...] + y[2 * M:RH]
        x2a_s[...] = x2a_new
        xin0 = xb_s[...]
        xin1 = jnp.where(first, y_old, x2a_new)
        hb = jnp.concatenate([_ln(xin0).astype(BF16), _ln(xin1).astype(BF16)], axis=0)
        for j in range(FT):
            glu_chunk(hb, j)
        z = glu_down(RB)
        res0 = xin0 + z[0:SEG]
        res1 = xin1 + z[SEG:RB]

        @pl.when(first)
        def _():
            x2_s[...] = res0
            _store_tiles(ha_s, 2 * M + SEG, _ln(res0).astype(BF16))
            out_copy(t - 2).wait()
            ost_s[0] = res1.astype(BF16)
            out_copy(t).start()

        @pl.when(jnp.logical_not(first))
        def _():
            out_copy(t - 2).wait()
            ost_s[1] = res0.astype(BF16)
            out_copy(t).start()
            out_copy(t - 1).wait()
            ost_s[0] = res1.astype(BF16)
            out_copy(t + 1).start()

    def x_next(t):
        seg = jnp.minimum(t, NSEG - 1)
        return pltpu.make_async_copy(x_hbm.at[pl.ds(pl.multiple_of(seg * SEG, SEG), SEG)],
                                     xr_s.at[t & (XR - 1)], sem_x.at[t & (XR - 1)])

    def head_body(t, carry):
        x_copy(t + XPF).start()
        head_step(t)
        return carry

    def pre_body_step(t, carry):
        @pl.when(t >= 5)
        def _():
            out_copy(t - 2).wait()

        @pl.when(t + 1 >= PRE0 + NPRE)
        def _():
            x_copy(t + 1).wait()
        x_copy(t + XPF).start()
        full_step(t, True)
        out_copy(t).start()
        return carry

    def full_body(t, carry):
        out_copy(t - 2).wait()
        x_next(t + 1).wait()
        x_next(t + XPF).start()
        full_step(t, False)
        out_copy(t).start()
        return carry

    def tail_body(t, carry):
        tail_step(t)
        return carry

    jax.lax.fori_loop(0, 2, head_body, 0)
    x_copy(PRE0 + XPF).start()
    full_step(PRE0, True, with_glu=False)
    jax.lax.fori_loop(PRE0 + 1, PRE0 + NPRE, pre_body_step, 0)
    jax.lax.fori_loop(PRE0 + NPRE, NSEG, full_body, 0)
    jax.lax.fori_loop(NSEG, NSEG + 2, tail_body, 0)
    for s in range(NSEG + 1, NSEG + XPF):
        x_next(s).wait()
    out_copy(NSTEP - 2).wait()
    out_copy(NSTEP - 1).wait()


@jax.jit
def pallas_interleave_layers__memory_aug_recurrent_mem_tr__glu_gated_glu__prompt_kernel(A_x, A_mem0, A_Wq, A_Wk, A_Wv, A_Wo, A_seg_len, B_x, B_w_gate, B_w_up, B_w_down):
    x = A_x.reshape(S, D)
    mem0 = A_mem0.reshape(M, D)
    wo = A_Wo.reshape(H * DH, D)
    any_spec = pl.BlockSpec(memory_space=pl.ANY)
    out = pl.pallas_call(
        _kernel,
        out_shape=jax.ShapeDtypeStruct((S, D), BF16),
        in_specs=[any_spec] * 9,
        out_specs=any_spec,
        scratch_shapes=[
            pltpu.VMEM((XR, SEG, D), BF16),
            pltpu.VMEM((M, D), BF16),
            pltpu.VMEM((H, D // 2, DH), U32),
            pltpu.VMEM((H, D // 2, DH), U32),
            pltpu.VMEM((H, D // 2, DH), U32),
            pltpu.VMEM((KT, H * DH // 2, 128), U32),
            pltpu.VMEM((FT, D // 2, 128), U32),
            pltpu.VMEM((FT, D // 2, 128), U32),
            pltpu.VMEM((KT, FF // 2, 128), U32),
            pltpu.VMEM((2 * NCH, DCH, H, DH), BF16),
            pltpu.VMEM((H * DH, D), BF16),
            pltpu.VMEM((D, FF), BF16),
            pltpu.VMEM((D, FF), BF16),
            pltpu.VMEM((FF, D), BF16),
            pltpu.VMEM((KT, RA // 2, 128), U32),
            pltpu.VMEM((KT, RB // 2, 128), U32),
            pltpu.VMEM((KT, NPRE * SEG // 2, 128), U32),
            pltpu.VMEM((3, H, NPRE * SEG, DH), F32),
            pltpu.VMEM((H, RA // 2, 128), U32),
            pltpu.VMEM((FT, RB // 2, 128), U32),
            pltpu.VMEM((SEG, D), F32),
            pltpu.VMEM((SEG, D), F32),
            pltpu.VMEM((SEG, D), F32),
            pltpu.VMEM((SEG, D), F32),
            pltpu.VMEM((2, SEG, D), BF16),
            pltpu.VMEM((RA, RA), F32),
            pltpu.SemaphoreType.DMA((XR,)),
            pltpu.SemaphoreType.DMA,
            pltpu.SemaphoreType.DMA((2 * NCH,)),
            pltpu.SemaphoreType.DMA((3 + NQ,)),
            pltpu.SemaphoreType.DMA((2,)),
        ],
        compiler_params=pltpu.CompilerParams(vmem_limit_bytes=126 * 1024 * 1024, disable_bounds_checks=True, disable_semaphore_checks=True),
    )(x, mem0, A_Wq, A_Wk, A_Wv, wo, B_w_gate, B_w_up, B_w_down)
    return out.reshape(1, S, D)
```
